```python
import jax
import jax.numpy as jnp

def _softmax(x, axis=-1):
    return jax.nn.softmax(x, axis=axis)

def _gelu(x):
    return jax.nn.gelu(x, approximate=True)

def _silu(x):
    return jax.nn.silu(x)

def _sigmoid(x):
    return jax.nn.sigmoid(x)

def _layernorm(x, axis=-1, eps=1e-05):
    m = jnp.mean(x, axis=axis, keepdims=True)
    v = jnp.var(x, axis=axis, keepdims=True)
    return (x - m) / jnp.sqrt(v + eps)

def _scatter_add(tgt, idx, src, axis=0):
    return tgt.at[idx].add(src)

def _segment_sum(src, seg, n):
    return jax.ops.segment_sum(src, seg, n)

class _Rng:

    def __init__(self, key):
        self._k = key

    def _next(self):
        self._k, sub = jax.random.split(self._k)
        return sub

    def normal(self, shape):
        return jax.random.normal(self._next(), shape, dtype=jnp.bfloat16)

    def randint(self, lo, hi, shape):
        return jax.random.randint(self._next(), shape, lo, hi, dtype=jnp.int32)

    def uniform(self, shape, lo=0.0, hi=1.0):
        return jax.random.uniform(self._next(), shape, jnp.bfloat16, lo, hi)

    def permutation(self, n):
        return jax.random.permutation(self._next(), n)
kernel_name = 'adaLN_cond__sliding_block_cached__mixer_token_mlp__decode'

def setup_inputs():
    _rng = _Rng(jax.random.key(int.from_bytes(__import__("os").urandom(4), "little")))
    _w = lambda a: (lambda t: t.astype(jnp.bfloat16) if jnp.issubdtype(t.dtype, jnp.floating) else t)(jnp.asarray(a))

    def _A_setup():
        B, Sq, D = (1, 1, 640)
        Hq, Hkv, Sk, Dh = (32, 32, 32768, 192)
        assert Hq % Hkv == 0, (Hq, Hkv)
        return {'x': _w((lambda *s: _rng.normal(s) * 0.05)(B, Sq, D)), 'k_cache': _w((lambda *s: _rng.normal(s) * 0.05)(B, Hkv, Sk, Dh)), 'v_cache': _w((lambda *s: _rng.normal(s) * 0.05)(B, Hkv, Sk, Dh)), 'wq': _w((lambda *s: _rng.normal(s) * 0.05)(D, Hq * Dh) * D ** (-0.5)), 'wo': _w((lambda *s: _rng.normal(s) * 0.05)(Hq * Dh, D) * (Hq * Dh) ** (-0.5))}
    _A_in = _A_setup()

    def _B_setup():
        B, S, D, F = (1, 1, 640, 1536)
        return {'x': _w((lambda *s: _rng.normal(s) * 0.05)(B, S, D)), 'w1': _w((lambda *s: _rng.normal(s) * 0.05)(S, F) * S ** (-0.5)), 'b1': _w((lambda *s: _rng.normal(s) * 0.05)(F) * 0.02), 'w2': _w((lambda *s: _rng.normal(s) * 0.05)(F, S) * F ** (-0.5)), 'b2': _w((lambda *s: _rng.normal(s) * 0.05)(S) * 0.02)}
    _B_in = _B_setup()
    return {'A_x': _A_in['x'], 'A_k_cache': _A_in['k_cache'], 'A_v_cache': _A_in['v_cache'], 'A_wq': _A_in['wq'], 'A_wo': _A_in['wo'], 'B_x': _B_in['x'], 'B_w1': _B_in['w1'], 'B_b1': _B_in['b1'], 'B_w2': _B_in['w2'], 'B_b2': _B_in['b2'], 'c': _w((lambda *s: _rng.normal(s) * 0.05)(1, 640)), 'w_mod': _w((lambda *s: _rng.normal(s) * 0.05)(640, 6 * 640) * 640 ** (-0.5))}

def reference(A_x, A_k_cache, A_v_cache, A_wq, A_wo, B_x, B_w1, B_b1, B_w2, B_b2, c, w_mod):

    def _A_ref(x, k_cache, v_cache, wq, wo):
        B, Sq, D = x.shape
        Hq, Dh = (32, 192)
        Hkv, Sk = (k_cache.shape[1], k_cache.shape[2])
        W = min(4096, max(256, Sk // 4))
        rep = Hq // Hkv
        q = (lambda x, *d: x.transpose(*d))((x @ wq).reshape(B, Sq, Hq, Dh), 0, 2, 1, 3)
        k = jnp.repeat(k_cache[:, :, Sk - W:, :], rep, axis=1)
        v = jnp.repeat(v_cache[:, :, Sk - W:, :], rep, axis=1)
        scores = jnp.einsum('bhqd,bhkd->bhqk', q, k) * Dh ** (-0.5)
        p = _softmax(scores, axis=-1)
        o = jnp.einsum('bhqk,bhkd->bhqd', p, v)
        return (lambda x, *d: x.transpose(*d))(o, 0, 2, 1, 3).reshape(B, Sq, Hq * Dh) @ wo

    def _B_ref(x, w1, b1, w2, b2):
        B, S, D = x.shape
        h = _layernorm(x, axis=-1)
        u = jnp.einsum('bsd,sf->bdf', h, w1) + b1
        u = _gelu(u)
        y = jnp.einsum('bdf,fs->bds', u, w2) + b2
        return (lambda x, *d: x.transpose(*d))(y, 0, 2, 1)
    x = A_x
    mod = (_silu(c) @ w_mod).reshape(c.shape[0], 6, 1, -1)
    sa, ca, ga, sb, cb, gb = (mod[:, 0].copy(), mod[:, 1].copy(), mod[:, 2].copy(), mod[:, 3].copy(), mod[:, 4].copy(), mod[:, 5].copy())
    h = _layernorm(x, axis=-1) * (1 + ca) + sa
    x = x + ga * _A_ref(h, A_k_cache, A_v_cache, A_wq, A_wo)
    h = _layernorm(x, axis=-1) * (1 + cb) + sb
    x = x + gb * _B_ref(h, B_w1, B_b1, B_w2, B_b2)
    return x
```

```python
import functools
import math

import jax
import jax.numpy as jnp
import jax.experimental.pallas as pl
import jax.experimental.pallas.tpu as pltpu

_F32 = jnp.float32
_BF16 = jnp.bfloat16

_EPS = 1e-05
_GROUP = 8


def _layernorm(v):
    n = v.shape[-1]
    m = jnp.sum(v, axis=-1, keepdims=True) * (1.0 / n)
    d = v - m
    var = jnp.sum(d * d, axis=-1, keepdims=True) * (1.0 / n)
    return d * jax.lax.rsqrt(var + _EPS)


def _kernel(
    x_hbm, k_hbm, v_hbm, wq_hbm, wo_hbm, w1_hbm, b1_hbm, w2_hbm, b2_hbm, c_hbm, wm_hbm,
    o_ref,
    x_v, c_v, w1_v, b1_v, w2_v, b2_v, wm_v, wq_v, wo_v, ring, qbd, s_acc, p_buf, linv, acc,
    small_sems, big_sems, ring_sems,
    *, D, H, Dh, Sk, W, F, R, NS,
):
    HD = H * Dh
    GR = _GROUP * Dh
    NG = H // _GROUP
    NC = HD // R
    CPG = GR // R
    scale = Dh ** (-0.5)

    small = [(c_hbm, c_v), (x_hbm, x_v), (w1_hbm, w1_v), (b1_hbm, b1_v), (w2_hbm, w2_v), (b2_hbm, b2_v)]
    small_cp = [pltpu.make_async_copy(s, d, small_sems.at[i]) for i, (s, d) in enumerate(small)]

    def wm_cp(j):
        return pltpu.make_async_copy(
            wm_hbm.at[:, pl.ds(j * D, D)], wm_v.at[:, pl.ds(j * D, D)], big_sems.at[j])

    wq_cp = pltpu.make_async_copy(wq_hbm, wq_v, big_sems.at[6])
    wo_cp = pltpu.make_async_copy(wo_hbm, wo_v, big_sems.at[7])

    def ring_cp(src, j, slot):
        return pltpu.make_async_copy(
            src.at[pl.ds(j * R, R), pl.ds(Sk - W, W)], ring.at[slot], ring_sems.at[slot])

    wm_cp(0).start()
    wm_cp(1).start()
    for cp in small_cp:
        cp.start()
    wq_cp.start()
    for j in range(NS):
        ring_cp(k_hbm, j, j).start()
    wo_cp.start()

    for cp in small_cp:
        cp.wait()
    c = c_v[...].astype(_F32)
    sc = c * jax.nn.sigmoid(c)
    sc8 = jnp.broadcast_to(sc, (8, D)).astype(_BF16)
    x = x_v[0].astype(_F32)
    xn = _layernorm(x)

    def mod(j):
        return jnp.dot(sc8, wm_v[:, j * D:(j + 1) * D], preferred_element_type=_F32)

    wm_cp(0).wait()
    wm_cp(1).wait()
    h = xn * (1.0 + mod(1)) + mod(0)
    h = h.astype(_BF16)

    wq_cp.wait()
    row = jax.lax.broadcasted_iota(jnp.int32, (_GROUP, GR), 0) * Dh
    col = jax.lax.broadcasted_iota(jnp.int32, (_GROUP, GR), 1)
    diag = (col >= row) & (col < row + Dh)
    for g in range(NG):
        q = jnp.dot(h, wq_v[:, g * GR:(g + 1) * GR], preferred_element_type=_F32)
        q = jnp.where(diag, q, 0.0)
        for j in range(CPG):
            qbd[g * CPG + j] = q[:, j * R:(j + 1) * R]
    s_acc[...] = jnp.zeros(s_acc.shape, _F32)
    acc[...] = jnp.zeros(acc.shape, _F32)

    def k_body(j, carry):
        slot = j % NS
        ring_cp(k_hbm, j, slot).wait()
        g = j // CPG
        s_acc[g] += jnp.dot(qbd[j].astype(_BF16), ring[slot], preferred_element_type=_F32)

        @pl.when(j + NS < NC)
        def _():
            ring_cp(k_hbm, j + NS, slot).start()

        @pl.when(j + NS >= NC)
        def _():
            ring_cp(v_hbm, j + NS - NC, slot).start()
        return carry

    jax.lax.fori_loop(0, NC, k_body, 0)

    for g in range(NG):
        s = s_acc[g]
        m = jnp.max(s, axis=-1, keepdims=True)
        p = jnp.exp((s - m) * scale)
        l = jnp.sum(p, axis=-1, keepdims=True)
        p_buf[g] = p
        linv[g] = jnp.broadcast_to(1.0 / l, (_GROUP, 128))

    wo_cp.wait()

    rowR = jax.lax.broadcasted_iota(jnp.int32, (_GROUP, R), 0) * Dh
    colR = jax.lax.broadcasted_iota(jnp.int32, (_GROUP, R), 1)

    def v_body(j, carry):
        slot = (j + NC) % NS
        ring_cp(v_hbm, j, slot).wait()
        g = j // CPG
        o = jax.lax.dot_general(
            p_buf[g].astype(_BF16), ring[slot], (((1,), (1,)), ((), ())),
            preferred_element_type=_F32)
        cg = colR + (j - g * CPG) * R
        o = jnp.where((cg >= rowR) & (cg < rowR + Dh), o * linv[g][:, 0:1], 0.0)
        r0 = pl.multiple_of(j * R, R)
        acc[...] += jnp.dot(o.astype(_BF16), wo_v[pl.ds(r0, R), :], preferred_element_type=_F32)

        @pl.when(j + NS < NC)
        def _():
            ring_cp(v_hbm, j + NS, slot).start()

        @pl.when(j + NS == NC)
        def _():
            for jj in range(2, 6):
                wm_cp(jj).start()
        return carry

    jax.lax.fori_loop(0, NC, v_body, 0)

    attn = jnp.sum(acc[...], axis=0, keepdims=True)
    wm_cp(2).wait()
    x1 = x + mod(2)[0:1] * attn
    x1n = _layernorm(x1)
    wm_cp(3).wait()
    wm_cp(4).wait()
    h2 = x1n * (1.0 + mod(4)[0:1]) + mod(3)[0:1]
    h3 = _layernorm(h2)

    w1 = w1_v[...].astype(_F32)
    w2 = w2_v[...].astype(_F32)
    b1 = b1_v[...].astype(_F32)
    k0 = math.sqrt(2.0 / math.pi)
    k1 = k0 * 0.044715
    y = jnp.zeros((8, D), _F32)
    sub = jax.lax.broadcasted_iota(jnp.int32, (128, 128), 0)
    for i in range(F // 128):
        blk = jnp.where(sub == 0, w1[:, i * 128:(i + 1) * 128],
                        jnp.where(sub == 1, b1[i:i + 1, :],
                                  jnp.where(sub == 2, w2[:, i * 128:(i + 1) * 128], 0.0)))
        bt = blk.T
        u = bt[:, 0:1] * h3 + bt[:, 1:2]
        z = u * (k0 + k1 * (u * u))
        gl = (0.5 * u) * (1.0 + jnp.tanh(z)) * bt[:, 2:3]
        y = y + jnp.sum(gl.reshape(16, 8, D), axis=0)
    y = jnp.sum(y, axis=0, keepdims=True) + b2_v[...].astype(_F32)
    wm_cp(5).wait()
    out = x1 + mod(5)[0:1] * y
    o_ref[0] = out.astype(o_ref.dtype)


@jax.jit
def pallas_adaLN_cond__sliding_block_cached__mixer_token_mlp__decode_kernel(
    A_x: jax.Array,
    A_k_cache: jax.Array,
    A_v_cache: jax.Array,
    A_wq: jax.Array,
    A_wo: jax.Array,
    B_x: jax.Array,
    B_w1: jax.Array,
    B_b1: jax.Array,
    B_w2: jax.Array,
    B_b2: jax.Array,
    c: jax.Array,
    w_mod: jax.Array,
):
    B, Sq, D = A_x.shape
    _, H, Sk, Dh = A_k_cache.shape
    F = B_w1.shape[1]
    assert B == 1 and Sq == 1 and B_w1.shape[0] == 1
    W = min(4096, max(256, Sk // 4))
    R = 256
    NS = 4
    HD = H * Dh

    kt = jnp.swapaxes(A_k_cache, 2, 3).reshape(HD, Sk)
    vt = jnp.swapaxes(A_v_cache, 2, 3).reshape(HD, Sk)
    b1 = B_b1.reshape(F // 128, 128)
    w2 = B_w2.reshape(1, F)
    b2 = B_b2.reshape(1, 1)

    kernel = functools.partial(_kernel, D=D, H=H, Dh=Dh, Sk=Sk, W=W, F=F, R=R, NS=NS)
    NG = H // _GROUP
    scratch = [
        pltpu.VMEM((1, 1, D), _BF16),
        pltpu.VMEM((1, D), _BF16),
        pltpu.VMEM((1, F), _BF16),
        pltpu.VMEM((F // 128, 128), _BF16),
        pltpu.VMEM((1, F), _BF16),
        pltpu.VMEM((1, 1), _BF16),
        pltpu.VMEM((D, 6 * D), _BF16),
        pltpu.VMEM((D, HD), _BF16),
        pltpu.VMEM((HD, D), _BF16),
        pltpu.VMEM((NS, R, W), _BF16),
        pltpu.VMEM((HD // R, _GROUP, R), _F32),
        pltpu.VMEM((NG, _GROUP, W), _F32),
        pltpu.VMEM((NG, _GROUP, W), _F32),
        pltpu.VMEM((NG, _GROUP, 128), _F32),
        pltpu.VMEM((_GROUP, D), _F32),
        pltpu.SemaphoreType.DMA((6,)),
        pltpu.SemaphoreType.DMA((8,)),
        pltpu.SemaphoreType.DMA((NS,)),
    ]
    return pl.pallas_call(
        kernel,
        out_shape=jax.ShapeDtypeStruct(A_x.shape, A_x.dtype),
        in_specs=[pl.BlockSpec(memory_space=pl.ANY)] * 11,
        out_specs=pl.BlockSpec(memory_space=pltpu.VMEM),
        scratch_shapes=scratch,
        compiler_params=pltpu.CompilerParams(vmem_limit_bytes=64 * 1024 * 1024),
    )(A_x, kt, vt, A_wq, A_wo, B_w1, b1, w2, b2, c, w_mod)
```

```python
import functools
import math

import jax
import jax.numpy as jnp
import jax.experimental.pallas as pl
import jax.experimental.pallas.tpu as pltpu

_F32 = jnp.float32
_BF16 = jnp.bfloat16

_EPS = 1e-05
_GROUP = 8
_CH = 128
_UR = 16
_NU = _CH // _UR
_RING = 4
_LAG = 2
_NSW = 8


def _layernorm(v):
    n = v.shape[-1]
    m = jnp.sum(v, axis=-1, keepdims=True) * (1.0 / n)
    d = v - m
    var = jnp.sum(d * d, axis=-1, keepdims=True) * (1.0 / n)
    return d * jax.lax.rsqrt(var + _EPS)


def _kernel(
    x_hbm, k_hbm, v_hbm, wq_hbm, wo_hbm, w1_hbm, b1_hbm, w2_hbm, b2_hbm, c_hbm, wm_hbm,
    o_ref,
    x_v, c_v, w1_v, b1_v, w2_v, b2_v, wm_v, wq_v, wo_v, ring, qbd, s_acc, p_buf, linv, acc,
    mod_v, h_v, sc_v, wcol,
    small_sems, w_sems, kv_sems, g_sems,
    *, D, H, Dh, Sk, W, F,
):
    HD = H * Dh
    GR = _GROUP * Dh
    NG = H // _GROUP
    NCH = HD // _CH
    CPG = GR // _CH
    CW = W // _NU
    scale = Dh ** (-0.5)
    PA, PP = 1792, 512

    def kv_piece(src, c, slot, u, c0, nc):
        r = c * _CH + u * _UR
        if not isinstance(r, int):
            r = pl.multiple_of(r, _UR)
        return pltpu.make_async_copy(
            src.at[pl.ds(r, _UR), pl.ds(Sk - W + c0, nc)],
            ring.at[slot, pl.ds(u * _UR, _UR), pl.ds(c0, nc)], kv_sems.at[u])

    def kv_head(src, c, slot, u):
        kv_piece(src, c, slot, u, 0, PA).start(priority=1)
        kv_piece(src, c, slot, u, PA, PP).start(priority=0)

    def kv_tail(src, c, slot, u):
        kv_piece(src, c, slot, u, PA + PP, W - PA - PP).start(priority=1)

    def kv_wait(slot, u):
        kv_piece(k_hbm, 0, slot, u, 0, W).wait()

    def w_piece(i, p):
        src, dst, r0, nr, c0, nc, _ = p
        return pltpu.make_async_copy(
            src.at[pl.ds(r0, nr), pl.ds(c0, nc)], dst.at[pl.ds(r0, nr), pl.ds(c0, nc)],
            w_sems.at[i % _NSW])

    def strided_units(src, dst, nrows, rstride, nr, c_lo, c_hi, cw, nseg, p0c, p0r):
        segs = [(a + j, c) for c in range(c_lo, c_hi, cw) for j in range(0, rstride, nr)
                for a in range(0, nrows, rstride)]
        units = []
        for s in range(0, len(segs), nseg):
            u = []
            grp = segs[s:s + nseg]
            for k, (r, c) in enumerate(grp):
                if p0c:
                    u.append((src, dst, r, nr, c, cw - p0c, 1))
                elif k == len(grp) - 1:
                    u.append((src, dst, r, nr - p0r, c, cw, 1))
                else:
                    u.append((src, dst, r, nr, c, cw, 1))
            for k, (r, c) in enumerate(grp):
                if p0c:
                    u.append((src, dst, r, nr, c + cw - p0c, p0c, 0))
                elif k == len(grp) - 1:
                    u.append((src, dst, r + nr - p0r, p0r, c, cw, 0))
            units.append(u)
        return units

    units_a = strided_units(wm_hbm, wm_v, D, 80, 8, 0, 3 * D, 3 * D, 4, 256, 0)
    units_q = strided_units(wq_hbm, wq_v, D, 64, 8, 0, HD, 2048, 4, 256, 0)
    units_o = strided_units(wo_hbm, wo_v, HD, 384, 48, 0, D, D, 2, 0, 16)
    pre = units_a + units_q + units_o
    units_s = [[(wm_hbm, wm_v, r, 32, 3 * D, 2 * D - 128, 1), (wm_hbm, wm_v, r, 32, 5 * D - 128, 128, 0)]
               for r in range(0, D, 32)]

    def w_start(units, i):
        for p in units[i]:
            w_piece(i, p).start(priority=p[-1])

    def w_wait(units, i):
        for p in units[i]:
            w_piece(i, p).wait()

    small = [(c_hbm, c_v), (x_hbm, x_v), (w1_hbm, w1_v), (b1_hbm, b1_v), (w2_hbm, w2_v), (b2_hbm, b2_v)]
    small_cp = [pltpu.make_async_copy(s, d, small_sems.at[i]) for i, (s, d) in enumerate(small)]
    gb_cp = pltpu.make_async_copy(wm_hbm.at[:, pl.ds(5 * D, D)], wm_v.at[:, pl.ds(5 * D, D)], g_sems.at[0])

    def prep_small():
        for cp in small_cp:
            cp.wait()
        c = c_v[...].astype(_F32)
        sc_v[...] = jnp.broadcast_to(c * jax.nn.sigmoid(c), (8, D))
        s_acc[...] = jnp.zeros(s_acc.shape, _F32)
        acc[...] = jnp.zeros(acc.shape, _F32)

    def prep_mlp(i):
        sub = jax.lax.broadcasted_iota(jnp.int32, (128, 128), 0)
        w1 = w1_v[:, i * 128:(i + 1) * 128].astype(_F32)
        w2 = w2_v[:, i * 128:(i + 1) * 128].astype(_F32)
        b1 = b1_v[...].astype(_F32)[i:i + 1, :]
        blk = jnp.where(sub == 0, w1, jnp.where(sub == 1, b1, jnp.where(sub == 2, w2, 0.0)))
        wcol[i * 128:(i + 1) * 128, :] = blk.T

    def mod_tile(t):
        mod_v[:, t * 128:(t + 1) * 128] = jnp.dot(
            sc_v[...].astype(_BF16), wm_v[:, t * 128:(t + 1) * 128], preferred_element_type=_F32)

    def make_h():
        x = x_v[0].astype(_F32)
        h_v[...] = _layernorm(x) * (1.0 + mod_v[:, D:2 * D]) + mod_v[:, 0:D]

    def q_tile(t):
        q = jnp.dot(h_v[...].astype(_BF16), wq_v[:, t * 128:(t + 1) * 128], preferred_element_type=_F32)
        lo = jax.lax.broadcasted_iota(jnp.int32, (_GROUP, _CH), 0) * Dh - (t % CPG) * _CH
        col = jax.lax.broadcasted_iota(jnp.int32, (_GROUP, _CH), 1)
        qbd[t] = jnp.where((col >= lo) & (col < lo + Dh), q, 0.0)

    nA, nQ, nO = len(units_a), len(units_q), len(units_o)
    work = {}
    work.setdefault(4, []).append(prep_small)
    for i in range(F // 128):
        work.setdefault(5 + i, []).append(functools.partial(prep_mlp, i))
    for t in range(3 * D // 128):
        work.setdefault(nA + t, []).append(functools.partial(mod_tile, t))
    work.setdefault(nA + 3 * D // 128, []).append(make_h)
    for t in range(NCH):
        work.setdefault(nA + nQ + t, []).append(functools.partial(q_tile, t))
    assert NCH <= nO and 5 + F // 128 <= nA

    for i in range(_NSW):
        w_start(pre, i)
    for cp in small_cp:
        cp.start()
    npre = len(pre)
    for i in range(npre):
        w_wait(pre, i)
        if i + _NSW < npre:
            w_start(pre, i + _NSW)
        else:
            u = i + _NSW - npre
            kv_head(k_hbm, 0, 0, u)
            if u >= _LAG:
                kv_tail(k_hbm, 0, 0, u - _LAG)
        for fn in work.get(i, ()):
            fn()

    def k_step(j, u):
        g = j // CPG
        cols = pl.ds(u * CW, CW)
        s_acc[g, :, cols] += jnp.dot(
            qbd[j].astype(_BF16), ring[j % _RING, :, cols], preferred_element_type=_F32)

    def softmax(g):
        s = s_acc[g]
        m = jnp.max(s, axis=-1, keepdims=True)
        p = jnp.exp((s - m) * scale)
        l = jnp.sum(p, axis=-1, keepdims=True)
        p_buf[g] = p
        linv[g] = jnp.broadcast_to(1.0 / l, (_GROUP, 128))

    def v_step(j, u):
        g = j // CPG
        cols = pl.ds(u * CW, CW)
        return jax.lax.dot_general(
            p_buf[g, :, cols].astype(_BF16), ring[(j + NCH) % _RING, :, cols], (((1,), (1,)), ((), ())),
            preferred_element_type=_F32)

    def v_finish(j, o):
        g = j // CPG
        lo = jax.lax.broadcasted_iota(jnp.int32, (_GROUP, _CH), 0) * Dh - (j - g * CPG) * _CH
        col = jax.lax.broadcasted_iota(jnp.int32, (_GROUP, _CH), 1)
        o = jnp.where((col >= lo) & (col < lo + Dh), o * linv[g], 0.0)
        r0 = j * _CH
        if not isinstance(r0, int):
            r0 = pl.multiple_of(r0, _CH)
        acc[...] += jnp.dot(o.astype(_BF16), wo_v[pl.ds(r0, _CH), :], preferred_element_type=_F32)

    def tick(cur, nxt, c, u):
        kv_wait(c % _RING, u)
        if nxt is not None:
            kv_head(nxt[0], nxt[1], (c + 1) % _RING, u)
        if u >= _LAG:
            if nxt is not None:
                kv_tail(nxt[0], nxt[1], (c + 1) % _RING, u - _LAG)
        else:
            kv_tail(cur[0], cur[1], c % _RING, u - _LAG + _NU)

    for u in range(_NU):
        tick((k_hbm, 0), (k_hbm, 1), 0, u)

    def k_body(c, carry):
        for u in range(_NU):
            tick((k_hbm, c), (k_hbm, c + 1), c, u)
            k_step(c - 1, u)

        @pl.when(c % CPG == 0)
        def _():
            softmax(c // CPG - 1)
        return carry

    jax.lax.fori_loop(1, NCH - 1, k_body, 0)
    for u in range(_NU):
        tick((k_hbm, NCH - 1), (v_hbm, 0), NCH - 1, u)
        k_step(NCH - 2, u)
    for u in range(_NU):
        tick((v_hbm, 0), (v_hbm, 1), NCH, u)
        k_step(NCH - 1, u)
    softmax(NG - 1)

    def v_body(j, carry):
        o = None
        for u in range(_NU):
            tick((v_hbm, j), (v_hbm, j + 1), NCH + j, u)
            part = v_step(j - 1, u)
            o = part if o is None else o + part
        v_finish(j - 1, o)
        return carry

    jax.lax.fori_loop(1, NCH - 1, v_body, 0)
    o = None
    for u in range(_NU):
        tick((v_hbm, NCH - 1), None, 2 * NCH - 1, u)
        w_start(units_s, u)
        part = v_step(NCH - 2, u)
        o = part if o is None else o + part
    v_finish(NCH - 2, o)

    nS = len(units_s)
    o = None
    x1 = x1n = None
    for i in range(nS):
        w_wait(units_s, i)
        if i + _NSW < nS:
            w_start(units_s, i + _NSW)
        elif i + _NSW == nS:
            gb_cp.start(priority=1)
        if i < _NU:
            part = v_step(NCH - 1, i)
            o = part if o is None else o + part
        if i == _NU:
            v_finish(NCH - 1, o)
        if i == _NU + 1:
            attn = jnp.sum(acc[...], axis=0, keepdims=True)
            x1 = x_v[0].astype(_F32) + mod_v[0:1, 2 * D:3 * D] * attn
            x1n = _layernorm(x1)
    sc8 = sc_v[...].astype(_BF16)
    sb_cb = jnp.dot(sc8, wm_v[:, 3 * D:5 * D], preferred_element_type=_F32)
    h2 = x1n * (1.0 + sb_cb[0:1, D:2 * D]) + sb_cb[0:1, 0:D]
    h3 = _layernorm(h2)

    k0 = math.sqrt(2.0 / math.pi)
    k1 = k0 * 0.044715
    y = jnp.zeros((8, D), _F32)
    for i in range(F // 128):
        bt = wcol[i * 128:(i + 1) * 128, :]
        u = bt[:, 0:1] * h3 + bt[:, 1:2]
        z = u * (k0 + k1 * (u * u))
        gl = (0.5 * u) * (1.0 + jnp.tanh(z)) * bt[:, 2:3]
        y = y + jnp.sum(gl.reshape(16, 8, D), axis=0)
    y = jnp.sum(y, axis=0, keepdims=True) + b2_v[...].astype(_F32)
    gb_cp.wait()
    gb = jnp.dot(sc8, wm_v[:, 5 * D:6 * D], preferred_element_type=_F32)
    out = x1 + gb[0:1] * y
    o_ref[0] = out.astype(o_ref.dtype)


@jax.jit
def pallas_adaLN_cond__sliding_block_cached__mixer_token_mlp__decode_kernel(
    A_x: jax.Array,
    A_k_cache: jax.Array,
    A_v_cache: jax.Array,
    A_wq: jax.Array,
    A_wo: jax.Array,
    B_x: jax.Array,
    B_w1: jax.Array,
    B_b1: jax.Array,
    B_w2: jax.Array,
    B_b2: jax.Array,
    c: jax.Array,
    w_mod: jax.Array,
):
    B, Sq, D = A_x.shape
    _, H, Sk, Dh = A_k_cache.shape
    F = B_w1.shape[1]
    assert B == 1 and Sq == 1 and B_w1.shape[0] == 1
    W = min(4096, max(256, Sk // 4))
    HD = H * Dh

    kt = jnp.swapaxes(A_k_cache, 2, 3).reshape(HD, Sk)
    vt = jnp.swapaxes(A_v_cache, 2, 3).reshape(HD, Sk)
    b1 = B_b1.reshape(F // 128, 128)
    w2 = B_w2.reshape(1, F)
    b2 = B_b2.reshape(1, 1)

    kernel = functools.partial(_kernel, D=D, H=H, Dh=Dh, Sk=Sk, W=W, F=F)
    NG = H // _GROUP
    scratch = [
        pltpu.VMEM((1, 1, D), _BF16),
        pltpu.VMEM((1, D), _BF16),
        pltpu.VMEM((1, F), _BF16),
        pltpu.VMEM((F // 128, 128), _BF16),
        pltpu.VMEM((1, F), _BF16),
        pltpu.VMEM((1, 1), _BF16),
        pltpu.VMEM((D, 6 * D), _BF16),
        pltpu.VMEM((D, HD), _BF16),
        pltpu.VMEM((HD, D), _BF16),
        pltpu.VMEM((_RING, _CH, W), _BF16),
        pltpu.VMEM((HD // _CH, _GROUP, _CH), _F32),
        pltpu.VMEM((NG, _GROUP, W), _F32),
        pltpu.VMEM((NG, _GROUP, W), _F32),
        pltpu.VMEM((NG, _GROUP, 128), _F32),
        pltpu.VMEM((_GROUP, D), _F32),
        pltpu.VMEM((8, 3 * D), _F32),
        pltpu.VMEM((8, D), _F32),
        pltpu.VMEM((8, D), _F32),
        pltpu.VMEM((F, 128), _F32),
        pltpu.SemaphoreType.DMA((6,)),
        pltpu.SemaphoreType.DMA((_NSW,)),
        pltpu.SemaphoreType.DMA((_NU,)),
        pltpu.SemaphoreType.DMA((1,)),
    ]
    return pl.pallas_call(
        kernel,
        out_shape=jax.ShapeDtypeStruct(A_x.shape, A_x.dtype),
        in_specs=[pl.BlockSpec(memory_space=pl.ANY)] * 11,
        out_specs=pl.BlockSpec(memory_space=pltpu.VMEM),
        scratch_shapes=scratch,
        compiler_params=pltpu.CompilerParams(
            vmem_limit_bytes=64 * 1024 * 1024, disable_bounds_checks=True),
    )(A_x, kt, vt, A_wq, A_wo, B_w1, b1, w2, b2, c, w_mod)
```

```python
import functools
import math

import jax
import jax.numpy as jnp
import jax.experimental.pallas as pl
import jax.experimental.pallas.tpu as pltpu

_F32 = jnp.float32
_BF16 = jnp.bfloat16

CFG = dict(nocompute=False, notail=False, UR=8, LAG=4, AH=20, PA=1792, PP=384, NSW=20, NST=4,
           OFFQ=17, OFFO=17, OFFM=28, WP0=3, NDEF=8, DAH=20, DAH0=14, dorder=(1, 2, 0), gbm=384, mergeln=False,
           plan='mmmmmmmmmmmm')

_EPS = 1e-05
_GROUP = 8
_CH = 128
_RING = 4
_WIN = 32


def _rects(ncols, t0, t1):
    tpr = ncols // 128
    out = []
    while t0 < t1:
        g, c = divmod(t0, tpr)
        if c == 0 and t1 - t0 >= tpr:
            n = (t1 - t0) // tpr
            out.append((g * 8, n * 8, 0, ncols))
            t0 += n * tpr
        else:
            e = min(tpr, c + (t1 - t0))
            out.append((g * 8, 8, c * 128, (e - c) * 128))
            t0 += e - c
    return out


def _layernorm(v):
    n = v.shape[-1]
    m = jnp.sum(v, axis=-1, keepdims=True) * (1.0 / n)
    d = v - m
    var = jnp.sum(d * d, axis=-1, keepdims=True) * (1.0 / n)
    return d * jax.lax.rsqrt(var + _EPS)


def _layernorm_shifted(d):
    n = d.shape[-1]
    m = jnp.sum(d, axis=-1, keepdims=True) * (1.0 / n)
    ms = jnp.sum(d * d, axis=-1, keepdims=True) * (1.0 / n)
    return (d - m) * jax.lax.rsqrt(jnp.maximum(ms - m * m, 0.0) + _EPS)


def _allsum8(v):
    v = v + pltpu.roll(v, 4, 0)
    v = v + pltpu.roll(v, 2, 0)
    return v + pltpu.roll(v, 1, 0)


def _kernel(
    x_hbm, k_hbm, v_hbm, wq_hbm, wo_hbm, w1_hbm, b1_hbm, w2_hbm, b2_hbm, c_hbm, wm_hbm,
    o_ref,
    x_v, c_v, w1_v, b1_v, w2_v, b2_v, wm_v, wq_v, wo_v, ring, qbd, s_acc, p_buf, linv, acc,
    mod_v, h_v, sc_v, w1b, b1b, ab_v, lin_v, scb, ocol,
    small_sems, w_sems, kv_sems, g_sems, d_sems,
    *, D, H, Dh, Sk, W, F, cfg,
):
    HD = H * Dh
    GR = _GROUP * Dh
    NG = H // _GROUP
    NCH = HD // _CH
    CPG = GR // _CH
    UR, LAG, NSW, AH = cfg['UR'], cfg['LAG'], cfg['NSW'], cfg['AH']
    NU = _CH // UR
    NST = cfg['NST']
    CW = W // NST
    TPS = NU // NST
    NT = D // 128
    NB = F // 128
    scale = Dh ** (-0.5)
    PA, PP = cfg['PA'], cfg['PP']
    compute = not cfg['nocompute']
    k0 = math.sqrt(2.0 / math.pi)
    alpha = (k0 * 0.044715) ** (1.0 / 3.0)
    NDEF = cfg['NDEF']
    DSTEP = 4

    assert NU <= AH + 1 and AH <= 2 * NU and AH - LAG > 0

    def kv_piece(src, j, c, u, c0, nc):
        r = j * _CH + u * UR
        if not isinstance(r, int):
            r = pl.multiple_of(r, UR)
        return pltpu.make_async_copy(
            src.at[pl.ds(r, UR), pl.ds(Sk - W + c0, nc)],
            ring.at[c % _RING, pl.ds(u * UR, UR), pl.ds(c0, nc)], kv_sems.at[(c % 2) * NU + u])

    def kv_issue(where, c, u):
        dc, uu = divmod(u, NU)
        t = where(dc)
        if t is not None:
            kv_piece(t[0], t[1], c + dc, uu, 0, PA).start(priority=1)
            kv_piece(t[0], t[1], c + dc, uu, PA, PP).start(priority=0)
        dc, uu = divmod(u - LAG, NU)
        t = where(dc) if dc >= 0 else None
        if t is not None:
            kv_piece(t[0], t[1], c + dc, uu, PA + PP, W - PA - PP).start(priority=1)

    def kv_wait(c, u):
        kv_piece(k_hbm, 0, c, u, 0, W).wait()

    def where_static(c):
        def f(dc):
            cc = c + dc
            if cc < NCH: return (k_hbm, cc)
            if cc < 2 * NCH: return (v_hbm, cc - NCH)
            return None
        return f

    def unit(src, dst, ncols, cmax, spans):
        tiles = [t for a, b in spans for t in range(a, b) if (t % (ncols // 128)) * 128 < cmax]
        n0 = cfg['WP0'] if len(tiles) > 2 * cfg['WP0'] else 0
        pieces = []
        for part, prio in ((tiles[:len(tiles) - n0], 1), (tiles[len(tiles) - n0:], 0)):
            i = 0
            while i < len(part):
                k = i
                while k + 1 < len(part) and part[k + 1] == part[k] + 1:
                    k += 1
                for r in _rects(ncols, part[i], part[k] + 1):
                    pieces.append((src, dst) + r + (prio,))
                i = k + 1
        return pieces

    def windows(src, dst, shape, off, cmax, skip=()):
        nt = shape[0] // 8 * (shape[1] // 128)
        starts = list(range(off - _WIN, nt, _WIN))
        out = []
        for b in range(8):
            for s in starts[b::8]:
                a, e = max(s, 0), min(s + _WIN, nt)
                spans = [(a, e)]
                for (h0, h1) in skip:
                    spans = [x for (p, q) in spans for x in ((p, min(q, h0)), (max(p, h1), q)) if x[0] < x[1]]
                u = unit(src, dst, shape[1], cmax, spans)
                if u:
                    out.append(u)
        return out

    def interleave(*lists):
        items = sorted(((k + 0.5) / len(p), n, k) for n, p in enumerate(lists) for k in range(len(p)))
        return [lists[n][k] for _, n, k in items]

    tpc = _CH // 8 * NT
    holes = [(j * DSTEP * tpc, (j * DSTEP + 1) * tpc) for j in range(NDEF)]
    units_mq = interleave(windows(wm_hbm, wm_v, (D, 6 * D), cfg['OFFM'], 5 * D),
                          windows(wq_hbm, wq_v, (D, HD), cfg['OFFQ'], HD))
    units_o = windows(wo_hbm, wo_v, (HD, D), cfg['OFFO'], D, holes)
    pre = units_mq + units_o
    units_d = []
    for p in cfg['dorder']:
        for (h0, h1) in holes:
            cuts = [h0] + [t for t in range(h0 + 1, h1) if t % _WIN == cfg['OFFO'] % _WIN] + [h1]
            assert len(cuts) == 4
            units_d.append(((cuts[p], cuts[p + 1]), unit(wo_hbm, wo_v, D, D, [(cuts[p], cuts[p + 1])])))

    def piece(p, sem):
        src, dst, r0, nr, c0, nc, _ = p
        return pltpu.make_async_copy(
            src.at[pl.ds(r0, nr), pl.ds(c0, nc)], dst.at[pl.ds(r0, nr), pl.ds(c0, nc)], sem)

    def w_start(i):
        for p in pre[i]:
            piece(p, w_sems.at[i % NSW]).start(priority=p[-1])

    def w_wait(i):
        for p in pre[i]:
            piece(p, w_sems.at[i % NSW]).wait()

    small = [(c_hbm, c_v), (x_hbm, x_v), (w1_hbm, w1_v), (b1_hbm, b1_v), (w2_hbm, w2_v), (b2_hbm, b2_v)]
    small_cp = [pltpu.make_async_copy(s, d, small_sems.at[i]) for i, (s, d) in enumerate(small)]
    gb_cp = pltpu.make_async_copy(wm_hbm.at[:, pl.ds(5 * D, D)], wm_v.at[:, pl.ds(5 * D, D)], g_sems.at[0])
    d_next = [0, 0]

    def d_issue(upto1, upto0):
        while d_next[0] < upto1:
            i = d_next[0]
            if i < len(units_d):
                for p in units_d[i][1]:
                    if p[-1] == 1:
                        piece(p, d_sems.at[i]).start(priority=1)
            elif i == len(units_d):
                gb_cp.start(priority=1)
            d_next[0] += 1
        while d_next[1] < min(upto0, len(units_d)):
            for p in units_d[d_next[1]][1]:
                if p[-1] == 0:
                    piece(p, d_sems.at[d_next[1]]).start(priority=0)
            d_next[1] += 1

    def prep_small():
        c = c_v[...].astype(_F32)
        sc = (c * jax.nn.sigmoid(c)).astype(_BF16).astype(_F32)
        sc_v[...] = jnp.broadcast_to(sc, (8, D))
        s_acc[...] = jnp.zeros(s_acc.shape, _F32)
        acc[...] = jnp.zeros(acc.shape, _F32)

    def prep_scb(t):
        scb[t * 128:(t + 1) * 128, :] = jnp.broadcast_to(sc_v[0:1, t * 128:(t + 1) * 128], (128, 128)).T

    def prep_mlp(i):
        w1 = w1_v[:, i * 128:(i + 1) * 128].astype(_F32)
        w2 = w2_v[:, i * 128:(i + 1) * 128].astype(_F32)
        b1 = b1_v[...].astype(_F32)[i:i + 1, :]
        w1b[i * 128:(i + 1) * 128, :] = jnp.broadcast_to(w1 * alpha, (128, 128)).T
        b1b[i * 128:(i + 1) * 128, :] = jnp.broadcast_to(b1 * alpha, (128, 128)).T
        a = 0.5 * w2 * w1
        b = 0.5 * w2 * b1
        a_hi = a.astype(_BF16).astype(_F32)
        b_hi = b.astype(_BF16).astype(_F32)
        sub = jax.lax.broadcasted_iota(jnp.int32, (8, 128), 0)
        ab_v[:, i * 128:(i + 1) * 128] = jnp.where(
            sub == 0, a_hi, jnp.where(sub == 1, a - a_hi, jnp.where(
                sub == 2, b_hi, jnp.where(sub == 3, b - b_hi, 0.0))))

    def prep_lin():
        sub = jax.lax.broadcasted_iota(jnp.int32, (8, 128), 0)
        tot = jnp.broadcast_to(jnp.sum(ab_v[...], axis=1, keepdims=True), (8, 128))
        lin_v[...] = tot + jnp.where(sub == 2, jnp.broadcast_to(b2_v[...].astype(_F32), (8, 128)), 0.0)

    def mod_tiles(t0, t1):
        mod_v[:, t0 * 128:t1 * 128] = jnp.dot(
            sc_v[...].astype(_BF16), wm_v[:, t0 * 128:t1 * 128], preferred_element_type=_F32)

    def make_h():
        x = jnp.broadcast_to(x_v[0].astype(_F32), (8, D))
        h_v[...] = _layernorm(x) * (1.0 + mod_v[:, D:2 * D]) + mod_v[:, 0:D]

    def diag_mask(j):
        lo = jax.lax.broadcasted_iota(jnp.int32, (_GROUP, _CH), 0) * Dh - (j % CPG) * _CH
        col = jax.lax.broadcasted_iota(jnp.int32, (_GROUP, _CH), 1)
        return (col >= lo) & (col < lo + Dh)

    def q_tile(j):
        if not compute: return
        c0 = j * _CH
        if not isinstance(c0, int):
            c0 = pl.multiple_of(c0, _CH)
        q = jnp.dot(h_v[...].astype(_BF16), wq_v[:, pl.ds(c0, _CH)], preferred_element_type=_F32)
        qbd[j % 2] = jnp.where(diag_mask(j), q, 0.0)

    nMQ = len(units_mq)
    work = {}
    if compute:
        items = [prep_small] + [functools.partial(prep_scb, t) for t in range(NT)]
        items += [functools.partial(prep_mlp, i) for i in range(NB)] + [prep_lin]
        for k, fn in enumerate(items):
            work[12 + 6 * k] = [fn]
        items = [functools.partial(mod_tiles, t, min(t + 2, 5 * NT)) for t in range(0, 5 * NT, 2)] + [make_h]
        for k, fn in enumerate(items):
            work[nMQ + 5 * k] = [fn]
        assert nMQ + 5 * len(items) <= len(pre)

    for i in range(NSW):
        w_start(i)
    for cp in small_cp:
        cp.start()
    npre = len(pre)
    for i in range(npre):
        w_wait(i)
        if i + NSW < npre:
            w_start(i + NSW)
        else:
            k = i + NSW - npre
            for u in range(k * AH // NSW, (k + 1) * AH // NSW):
                kv_issue(where_static(0), 0, u)
        if i == 8:
            for cp in small_cp:
                cp.wait()
        for fn in work.get(i, ()):
            fn()

    def k_step(j, u):
        if not compute: return
        g = j // CPG
        cols = pl.ds(u * CW, CW)
        s_acc[g, :, cols] += jnp.dot(
            qbd[j % 2].astype(_BF16), ring[j % _RING, :, cols], preferred_element_type=_F32)

    def softmax(g):
        if not compute: return
        s = s_acc[g]
        m = jnp.max(s, axis=-1, keepdims=True)
        p = jnp.exp((s - m) * scale)
        l = jnp.sum(p, axis=-1, keepdims=True)
        p_buf[g] = p
        linv[g] = jnp.broadcast_to(1.0 / l, (_GROUP, 128))

    def v_step(j, u, o):
        if not compute: return None
        g = j // CPG
        cols = pl.ds(u * CW, CW)
        part = jax.lax.dot_general(
            p_buf[g, :, cols].astype(_BF16), ring[(j + NCH) % _RING, :, cols], (((1,), (1,)), ((), ())),
            preferred_element_type=_F32)
        return part if o is None else part + o

    def v_finish(j, o):
        if not compute: return
        o = jnp.where(diag_mask(j), o * linv[j // CPG], 0.0).astype(_BF16)

        def now():
            r0 = j * _CH
            if not isinstance(r0, int):
                r0 = pl.multiple_of(r0, _CH)
            acc[...] += jnp.dot(o, wo_v[pl.ds(r0, _CH), :], preferred_element_type=_F32)

        def later():
            row = jnp.sum(o.astype(_F32), axis=0, keepdims=True)
            ocol[j // DSTEP] = jnp.broadcast_to(row, (_CH, _CH)).T

        if isinstance(j, int):
            later() if (j % DSTEP == 0 and j < DSTEP * NDEF) else now()
        else:
            deferred = jnp.logical_and(j % DSTEP == 0, j < DSTEP * NDEF)
            pl.when(deferred)(later)
            pl.when(jnp.logical_not(deferred))(now)

    def tick(where, c, u):
        kv_wait(c, u)
        kv_issue(where, c, u + AH)

    QAT = NU - 2
    for u in range(NU):
        tick(where_static(0), 0, u)
        if u == QAT: q_tile(0)

    def k_body(c, carry):
        for u in range(NU):
            tick(lambda dc: (k_hbm, c + dc), c, u)
            if u % TPS == 0: k_step(c - 1, u // TPS)
            if u == QAT: q_tile(c)

        @pl.when(c % CPG == 0)
        def _():
            softmax(c // CPG - 1)
        return carry

    jax.lax.fori_loop(1, NCH - 2, k_body, 0)
    for c in range(NCH - 2, NCH + 1):
        for u in range(NU):
            tick(where_static(c), c, u)
            if u % TPS == 0: k_step(c - 1, u // TPS)
            if u == QAT and c < NCH: q_tile(c)
    softmax(NG - 1)

    def v_body(j, carry):
        o = None
        for u in range(NU):
            tick(lambda dc: (v_hbm, j + dc), NCH + j, u)
            if u % TPS == 0: o = v_step(j - 1, u // TPS, o)
            if u == NU - 1: v_finish(j - 1, o)
        return carry

    jax.lax.fori_loop(1, NCH - 2, v_body, 0)
    nleft = AH - LAG + 1
    for j in range(NCH - 2, NCH):
        o = None
        for u in range(NU):
            tick(where_static(NCH + j), NCH + j, u)
            k = nleft - ((NCH - j) * NU - u) + 1
            if k > 0:
                d_issue(k * cfg['DAH'] // nleft, k * cfg['DAH0'] // nleft)
            if u % TPS == 0: o = v_step(j - 1, u // TPS, o)
        v_finish(j - 1, o)

    nD = len(units_d)
    accd = [None] * NT

    def d_work(i):
        t0, t1 = units_d[i][0]
        for (r0, nr, c0, nc) in _rects(D, t0, t1):
            oc = ocol[r0 // _CH // DSTEP, pl.ds(r0 % _CH, nr), :].reshape(nr // 8, 8, 128)
            for c in range(c0, c0 + nc, 128):
                w = wo_v[r0:r0 + nr, c:c + 128].astype(_F32).reshape(nr // 8, 8, 128)
                part = jnp.sum(w * oc, axis=0)
                accd[c // 128] = part if accd[c // 128] is None else accd[c // 128] + part

    st = {}
    o = None
    done = 0
    for i in range(nD):
        for p in units_d[i][1]:
            piece(p, d_sems.at[i]).wait()
        d_issue(i + 1 + cfg['DAH'], i + 1 + cfg['DAH0'])
        if not compute:
            continue
        if i == 0 or i == 4:
            for u in range((i // 4) * NST // 2, (i // 4 + 1) * NST // 2):
                o = v_step(NCH - 1, u, o)
        if i == 8:
            v_finish(NCH - 1, o)
        if i >= 10:
            while done <= i:
                d_work(done)
                done += 1
        if i == nD - 5:
            st['x'] = jnp.broadcast_to(x_v[0].astype(_F32), (8, D))
            st['ga'] = mod_v[:, 2 * D:3 * D]
            st['base'] = acc[...]
            x1 = st['x'] + st['ga'] * _allsum8(st['base'] + jnp.concatenate(accd, axis=1))
            st['m1'] = jnp.sum(x1, axis=-1, keepdims=True) * (1.0 / D)
            st['xs'] = st['x'] - st['m1']
            st['f'] = 1.0 + mod_v[:, 4 * D:5 * D]
            sb = mod_v[:, 3 * D:4 * D]
            st['g'] = sb - jnp.sum(sb, axis=-1, keepdims=True) * (1.0 / D)
    if not compute:
        gb_cp.wait()
        o_ref[...] = x_v[...]
        return
    ga_attn = st['ga'] * _allsum8(st['base'] + jnp.concatenate(accd, axis=1))
    x1 = st['x'] + ga_attn
    if cfg['notail']:
        gb_cp.wait()
        o_ref[0] = x1[0:1].astype(_BF16)
        return
    x1n = _layernorm_shifted(st['xs'] + ga_attn)
    h3 = _layernorm_shifted(x1n * st['f'] + st['g'])

    cst = k0 / alpha
    ys = [None] * NT
    for i in range(NB):
        wv = w1b[i * 128:(i + 1) * 128, :].reshape(16, 8, 128)
        bv = b1b[i * 128:(i + 1) * 128, :].reshape(16, 8, 128)
        for t in range(NT):
            v = wv * h3[:, t * 128:(t + 1) * 128] + bv
            th = jnp.tanh(v * (v * v + cst)).reshape(128, 128)
            part = jnp.dot(ab_v[:, i * 128:(i + 1) * 128], th, preferred_element_type=_F32)
            ys[t] = part if ys[t] is None else part + ys[t]
    lin = lin_v[...]
    yy = jnp.concatenate([y + lin for y in ys], axis=1)
    y = h3[0:1] * (yy[0:1] + yy[1:2]) + (yy[2:3] + yy[3:4])

    gb_cp.wait()
    gbm = cfg['gbm']
    gb = None
    if gbm > 0:
        gb = jnp.dot(sc_v[:, 0:gbm].astype(_BF16), wm_v[0:gbm, 5 * D:6 * D], preferred_element_type=_F32)[0:1]
    if gbm < D:
        n = D - gbm
        s3 = scb[gbm:D, :].reshape(n // 8, 8, 128)
        cols = []
        for c in range(5 * D, 6 * D, 128):
            w = wm_v[gbm:D, c:c + 128].astype(_F32).reshape(n // 8, 8, 128)
            cols.append(jnp.sum(jnp.sum(w * s3, axis=0), axis=0, keepdims=True))
        g2 = jnp.concatenate(cols, axis=1)
        gb = g2 if gb is None else gb + g2
    out = x1[0:1] + gb * y
    o_ref[0] = out.astype(o_ref.dtype)


def make(cfg):
  cfg = dict(CFG, **cfg)
  @jax.jit
  def pallas_adaLN_cond__sliding_block_cached__mixer_token_mlp__decode_kernel(
    A_x: jax.Array,
    A_k_cache: jax.Array,
    A_v_cache: jax.Array,
    A_wq: jax.Array,
    A_wo: jax.Array,
    B_x: jax.Array,
    B_w1: jax.Array,
    B_b1: jax.Array,
    B_w2: jax.Array,
    B_b2: jax.Array,
    c: jax.Array,
    w_mod: jax.Array,
  ):
    B, Sq, D = A_x.shape
    _, H, Sk, Dh = A_k_cache.shape
    F = B_w1.shape[1]
    assert B == 1 and Sq == 1 and B_w1.shape[0] == 1
    W = min(4096, max(256, Sk // 4))
    HD = H * Dh

    kt = jnp.swapaxes(A_k_cache, 2, 3).reshape(HD, Sk)
    vt = jnp.swapaxes(A_v_cache, 2, 3).reshape(HD, Sk)
    b1 = B_b1.reshape(F // 128, 128)
    w2 = B_w2.reshape(1, F)
    b2 = B_b2.reshape(1, 1)

    kernel = functools.partial(_kernel, D=D, H=H, Dh=Dh, Sk=Sk, W=W, F=F, cfg=cfg)
    NG = H // _GROUP
    scratch = [
        pltpu.VMEM((1, 1, D), _BF16),
        pltpu.VMEM((1, D), _BF16),
        pltpu.VMEM((1, F), _BF16),
        pltpu.VMEM((F // 128, 128), _BF16),
        pltpu.VMEM((1, F), _BF16),
        pltpu.VMEM((1, 1), _BF16),
        pltpu.VMEM((D, 6 * D), _BF16),
        pltpu.VMEM((D, HD), _BF16),
        pltpu.VMEM((HD, D), _BF16),
        pltpu.VMEM((_RING, _CH, W), _BF16),
        pltpu.VMEM((2, _GROUP, _CH), _F32),
        pltpu.VMEM((NG, _GROUP, W), _F32),
        pltpu.VMEM((NG, _GROUP, W), _F32),
        pltpu.VMEM((NG, _GROUP, 128), _F32),
        pltpu.VMEM((_GROUP, D), _F32),
        pltpu.VMEM((8, 5 * D), _F32),
        pltpu.VMEM((8, D), _F32),
        pltpu.VMEM((8, D), _F32),
        pltpu.VMEM((F, 128), _F32),
        pltpu.VMEM((F, 128), _F32),
        pltpu.VMEM((8, F), _F32),
        pltpu.VMEM((8, 128), _F32),
        pltpu.VMEM((D, 128), _F32),
        pltpu.VMEM((cfg['NDEF'], _CH, 128), _F32),
        pltpu.SemaphoreType.DMA((6,)),
        pltpu.SemaphoreType.DMA((cfg['NSW'],)),
        pltpu.SemaphoreType.DMA((2 * _CH // cfg['UR'],)),
        pltpu.SemaphoreType.DMA((1,)),
        pltpu.SemaphoreType.DMA((3 * cfg['NDEF'],)),
    ]
    return pl.pallas_call(
        kernel,
        out_shape=jax.ShapeDtypeStruct(A_x.shape, A_x.dtype),
        in_specs=[pl.BlockSpec(memory_space=pl.ANY)] * 11,
        out_specs=pl.BlockSpec(memory_space=pltpu.VMEM),
        scratch_shapes=scratch,
        compiler_params=pltpu.CompilerParams(
            vmem_limit_bytes=64 * 1024 * 1024, disable_bounds_checks=True,
            disable_semaphore_checks=True),
    )(A_x, kt, vt, A_wq, A_wo, B_w1, b1, w2, b2, c, w_mod)
  return pallas_adaLN_cond__sliding_block_cached__mixer_token_mlp__decode_kernel

pallas_adaLN_cond__sliding_block_cached__mixer_token_mlp__decode_kernel = make({})
```

```python
import functools
import math

import jax
import jax.numpy as jnp
import jax.experimental.pallas as pl
import jax.experimental.pallas.tpu as pltpu

_F32 = jnp.float32
_BF16 = jnp.bfloat16

_EPS = 1e-05
_GROUP = 8
_CH = 128
_RING = 4
_UR = 8
_NU = _CH // _UR
_AHEAD = 20
_LAG = 4
_PA, _PP = 1792, 384
_STEPS = 4
_WIN = 32
_WIN_HI = 3
_OFF_W, _OFF_M = 17, 28
_NDEF, _DSTEP = 8, 4
_DEF_HI_AHEAD = 16
_GB_MXU = 384


def _rects(ncols, t0, t1):
    tpr = ncols // 128
    out = []
    while t0 < t1:
        g, c = divmod(t0, tpr)
        if c == 0 and t1 - t0 >= tpr:
            n = (t1 - t0) // tpr
            out.append((g * 8, n * 8, 0, ncols))
            t0 += n * tpr
        else:
            e = min(tpr, c + (t1 - t0))
            out.append((g * 8, 8, c * 128, (e - c) * 128))
            t0 += e - c
    return out


def _unit(src, dst, ncols, cmax, spans):
    tiles = [t for a, b in spans for t in range(a, b) if (t % (ncols // 128)) * 128 < cmax]
    n_hi = _WIN_HI if len(tiles) > 2 * _WIN_HI else 0
    pieces = []
    for part, prio in ((tiles[:len(tiles) - n_hi], 1), (tiles[len(tiles) - n_hi:], 0)):
        i = 0
        while i < len(part):
            k = i
            while k + 1 < len(part) and part[k + 1] == part[k] + 1:
                k += 1
            pieces += [(src, dst) + r + (prio,) for r in _rects(ncols, part[i], part[k] + 1)]
            i = k + 1
    return pieces


def _windows(src, dst, shape, off, cmax, skip=()):
    nt = shape[0] // 8 * (shape[1] // 128)
    starts = list(range(off - _WIN, nt, _WIN))
    out = []
    for b in range(8):
        for s in starts[b::8]:
            spans = [(max(s, 0), min(s + _WIN, nt))]
            for h0, h1 in skip:
                spans = [x for p, q in spans for x in ((p, min(q, h0)), (max(p, h1), q)) if x[0] < x[1]]
            u = _unit(src, dst, shape[1], cmax, spans)
            if u:
                out.append(u)
    return out


def _interleave(*lists):
    items = sorted(((k + 0.5) / len(p), n, k) for n, p in enumerate(lists) for k in range(len(p)))
    return [lists[n][k] for _, n, k in items]


def _mean(v):
    return jnp.sum(v, axis=-1, keepdims=True) * (1.0 / v.shape[-1])


def _layernorm(v):
    d = v - _mean(v)
    return d * jax.lax.rsqrt(_mean(d * d) + _EPS)


def _allsum8(v):
    v = v + pltpu.roll(v, 4, 0)
    v = v + pltpu.roll(v, 2, 0)
    return v + pltpu.roll(v, 1, 0)


def _columns(row):
    return jnp.broadcast_to(row, (128, 128)).T


def _aligned(i, n):
    return i if isinstance(i, int) else pl.multiple_of(i, n)


def _kernel(
    x_hbm, k_hbm, v_hbm, wq_hbm, wo_hbm, w1_hbm, b1_hbm, w2_hbm, b2_hbm, c_hbm, wm_hbm,
    o_ref,
    x_v, c_v, w1_v, b1_v, w2_v, b2_v, wm_v, wq_v, wo_v, ring, qbd, s_acc, p_buf, linv, acc,
    mod_v, h_v, sc_v, w1b, b1b, ab_v, lin_v, scb, ocol, gsh, th_v, inf_v,
    small_sems, w_sems, kv_sems, g_sem, d_sems,
    *, D, H, Dh, Sk, W, F,
):
    HD = H * Dh
    NG = H // _GROUP
    NCH = HD // _CH
    CPG = _GROUP * Dh // _CH
    CW = W // _STEPS
    TPS = _NU // _STEPS
    NT = D // 128
    NB = F // 128
    scale = Dh ** (-0.5)
    k0 = math.sqrt(2.0 / math.pi)
    alpha = (k0 * 0.044715) ** (1.0 / 3.0)

    def kv_piece(src, j, c, u, c0, nc):
        r = _aligned(j * _CH + u * _UR, _UR)
        return pltpu.make_async_copy(
            src.at[pl.ds(r, _UR), pl.ds(Sk - W + c0, nc)],
            ring.at[c % _RING, pl.ds(u * _UR, _UR), pl.ds(c0, nc)],
            kv_sems.at[(c % 2) * _NU + u])

    def kv_issue(where, c, u):
        dc, uu = divmod(u, _NU)
        t = where(dc)
        if t is not None:
            kv_piece(t[0], t[1], c + dc, uu, 0, _PA).start(priority=1)
            kv_piece(t[0], t[1], c + dc, uu, _PA, _PP).start(priority=0)
        dc, uu = divmod(u - _LAG, _NU)
        t = where(dc) if dc >= 0 else None
        if t is not None:
            kv_piece(t[0], t[1], c + dc, uu, _PA + _PP, W - _PA - _PP).start(priority=1)

    def where_static(c):
        def where(dc):
            if c + dc < NCH:
                return (k_hbm, c + dc)
            if c + dc < 2 * NCH:
                return (v_hbm, c + dc - NCH)
            return None
        return where

    def tick(where, c, u):
        kv_piece(k_hbm, 0, c, u, 0, W).wait()
        kv_issue(where, c, u + _AHEAD)

    tpc = _CH // 8 * NT
    holes = [(j * _DSTEP * tpc, (j * _DSTEP + 1) * tpc) for j in range(_NDEF)]
    units_mq = _interleave(_windows(wm_hbm, wm_v, (D, 6 * D), _OFF_M, 5 * D),
                           _windows(wq_hbm, wq_v, (D, HD), _OFF_W, HD))
    pre = units_mq + _windows(wo_hbm, wo_v, (HD, D), _OFF_W, D, holes)
    units_d = []
    for p in (1, 2, 0):
        for h0, h1 in holes:
            cuts = [h0] + [t for t in range(h0 + 1, h1) if t % _WIN == _OFF_W] + [h1]
            assert len(cuts) == 4
            span = (cuts[p], cuts[p + 1])
            units_d.append((span, _unit(wo_hbm, wo_v, D, D, [span])))

    def piece(p, sem):
        src, dst, r0, nr, c0, nc, _ = p
        return pltpu.make_async_copy(
            src.at[pl.ds(r0, nr), pl.ds(c0, nc)], dst.at[pl.ds(r0, nr), pl.ds(c0, nc)], sem)

    def w_start(i):
        for p in pre[i]:
            piece(p, w_sems.at[i % _AHEAD]).start(priority=p[-1])

    def w_wait(i):
        for p in pre[i]:
            piece(p, w_sems.at[i % _AHEAD]).wait()

    small = [(c_hbm, c_v), (x_hbm, x_v), (w1_hbm, w1_v), (b1_hbm, b1_v), (w2_hbm, w2_v), (b2_hbm, b2_v)]
    small_cp = [pltpu.make_async_copy(s, d, small_sems.at[i]) for i, (s, d) in enumerate(small)]
    gb_cp = pltpu.make_async_copy(
        wm_hbm.at[:, pl.ds(5 * D, D)], wm_v.at[:, pl.ds(5 * D, D)], g_sem.at[0])
    d_next = [0, 0]

    def d_issue(upto_lo, upto_hi):
        while d_next[0] < upto_lo:
            i = d_next[0]
            if i < len(units_d):
                for p in units_d[i][1]:
                    if p[-1] == 1:
                        piece(p, d_sems.at[i]).start(priority=1)
            elif i == len(units_d):
                gb_cp.start(priority=1)
            d_next[0] += 1
        while d_next[1] < min(upto_hi, len(units_d)):
            i = d_next[1]
            for p in units_d[i][1]:
                if p[-1] == 0:
                    piece(p, d_sems.at[i]).start(priority=0)
            d_next[1] += 1

    def prep_small():
        c = c_v[...].astype(_F32)
        sc = (c * jax.nn.sigmoid(c)).astype(_BF16).astype(_F32)
        sc_v[...] = jnp.broadcast_to(sc, (8, D))
        s_acc[...] = jnp.zeros(s_acc.shape, _F32)
        acc[...] = jnp.zeros(acc.shape, _F32)
        inf_v[...] = jnp.full(inf_v.shape, jnp.inf, _F32)

    def prep_scb(r):
        scb[r - _GB_MXU:r - _GB_MXU + 128, :] = _columns(sc_v[0:1, r:r + 128])

    def prep_mlp(i):
        w1 = w1_v[:, i * 128:(i + 1) * 128].astype(_F32)
        w2 = w2_v[:, i * 128:(i + 1) * 128].astype(_F32)
        b1 = b1_v[...].astype(_F32)[i:i + 1, :]
        w1b[i * 128:(i + 1) * 128, :] = _columns(w1 * alpha)
        b1b[i * 128:(i + 1) * 128, :] = _columns(b1 * alpha)
        a = 0.5 * w2 * w1
        b = 0.5 * w2 * b1
        a_hi = a.astype(_BF16).astype(_F32)
        b_hi = b.astype(_BF16).astype(_F32)
        sub = jax.lax.broadcasted_iota(jnp.int32, (8, 128), 0)
        ab_v[:, i * 128:(i + 1) * 128] = jnp.where(
            sub == 0, a_hi, jnp.where(sub == 1, a - a_hi, jnp.where(
                sub == 2, b_hi, jnp.where(sub == 3, b - b_hi, 0.0))))

    def prep_lin():
        sub = jax.lax.broadcasted_iota(jnp.int32, (8, 128), 0)
        tot = jnp.broadcast_to(jnp.sum(ab_v[...], axis=1, keepdims=True), (8, 128))
        lin_v[...] = tot + jnp.where(sub == 2, jnp.broadcast_to(b2_v[...].astype(_F32), (8, 128)), 0.0)

    def mod_tiles(t0, t1):
        mod_v[:, t0 * 128:t1 * 128] = jnp.dot(
            sc_v[...].astype(_BF16), wm_v[:, t0 * 128:t1 * 128], preferred_element_type=_F32)

    def make_h():
        x = jnp.broadcast_to(x_v[0].astype(_F32), (8, D))
        h_v[...] = _layernorm(x) * (1.0 + mod_v[:, D:2 * D]) + mod_v[:, 0:D]
        sb = mod_v[:, 3 * D:4 * D]
        gsh[...] = sb - _mean(sb)

    work = {}
    items = [prep_small] + [functools.partial(prep_scb, r) for r in range(_GB_MXU, D, 128)]
    items += [functools.partial(prep_mlp, i) for i in range(NB)] + [prep_lin]
    for k, fn in enumerate(items):
        work[12 + 6 * k] = fn
    assert 12 + 6 * len(items) <= len(units_mq)
    items = [functools.partial(mod_tiles, t, min(t + 2, 5 * NT)) for t in range(0, 5 * NT, 2)] + [make_h]
    for k, fn in enumerate(items):
        work[len(units_mq) + 5 * k] = fn
    assert len(units_mq) + 5 * len(items) <= len(pre)

    for i in range(_AHEAD):
        w_start(i)
    for cp in small_cp:
        cp.start()
    for i in range(len(pre)):
        w_wait(i)
        if i + _AHEAD < len(pre):
            w_start(i + _AHEAD)
        else:
            kv_issue(where_static(0), 0, i + _AHEAD - len(pre))
        if i == 8:
            for cp in small_cp:
                cp.wait()
        if i in work:
            work[i]()

    def diag_mask(j):
        lo = jax.lax.broadcasted_iota(jnp.int32, (_GROUP, _CH), 0) * Dh - (j % CPG) * _CH
        col = jax.lax.broadcasted_iota(jnp.int32, (_GROUP, _CH), 1)
        return (col >= lo) & (col < lo + Dh)

    def q_tile(j):
        q = jnp.dot(h_v[...].astype(_BF16), wq_v[:, pl.ds(_aligned(j * _CH, _CH), _CH)],
                    preferred_element_type=_F32)
        qbd[j % 2] = jnp.where(diag_mask(j), q, 0.0)

    def k_step(j, s):
        cols = pl.ds(s * CW, CW)
        s_acc[j // CPG, :, cols] += jnp.dot(
            qbd[j % 2].astype(_BF16), ring[j % _RING, :, cols], preferred_element_type=_F32)

    def softmax(g):
        s = s_acc[g]
        m = jnp.max(s, axis=-1, keepdims=True)
        p = jnp.exp((s - m) * scale)
        p_buf[g] = p
        linv[g] = jnp.broadcast_to(1.0 / jnp.sum(p, axis=-1, keepdims=True), (_GROUP, 128))

    def v_step(j, s, o):
        cols = pl.ds(s * CW, CW)
        part = jax.lax.dot_general(
            p_buf[j // CPG, :, cols].astype(_BF16), ring[(j + NCH) % _RING, :, cols],
            (((1,), (1,)), ((), ())), preferred_element_type=_F32)
        return part if o is None else part + o

    def v_finish(j, o):
        o = jnp.where(diag_mask(j), o * linv[j // CPG], 0.0).astype(_BF16)

        def now():
            acc[...] += jnp.dot(o, wo_v[pl.ds(_aligned(j * _CH, _CH), _CH), :], preferred_element_type=_F32)

        def later():
            ocol[j // _DSTEP] = _columns(jnp.sum(o.astype(_F32), axis=0, keepdims=True))

        if isinstance(j, int):
            assert j >= _DSTEP * _NDEF
            now()
        else:
            deferred = jnp.logical_and(j % _DSTEP == 0, j < _DSTEP * _NDEF)
            pl.when(deferred)(later)
            pl.when(jnp.logical_not(deferred))(now)

    def k_chunk(where, c, first=False, last=False):
        for u in range(_NU):
            tick(where, c, u)
            if u % TPS == 0 and not first:
                k_step(c - 1, u // TPS)
            if u == _NU - 2 and not last:
                q_tile(c)

    def k_body(c, carry):
        k_chunk(lambda dc: (k_hbm, c + dc), c)

        @pl.when(c % CPG == 0)
        def _():
            softmax(c // CPG - 1)
        return carry

    k_chunk(where_static(0), 0, first=True)
    jax.lax.fori_loop(1, NCH - 2, k_body, 0)
    for c in range(NCH - 2, NCH + 1):
        k_chunk(where_static(c), c, last=c == NCH)
    softmax(NG - 1)

    def v_body(j, carry):
        o = None
        for u in range(_NU):
            tick(lambda dc: (v_hbm, j + dc), NCH + j, u)
            if u % TPS == 0:
                o = v_step(j - 1, u // TPS, o)
        v_finish(j - 1, o)
        return carry

    jax.lax.fori_loop(1, NCH - 2, v_body, 0)
    nleft = _AHEAD - _LAG + 1
    for j in range(NCH - 2, NCH):
        o = None
        for u in range(_NU):
            tick(where_static(NCH + j), NCH + j, u)
            k = nleft - ((NCH - j) * _NU - u) + 1
            if k > 0:
                d_issue(k * _AHEAD // nleft, k * _DEF_HI_AHEAD // nleft)
            if u % TPS == 0:
                o = v_step(j - 1, u // TPS, o)
        v_finish(j - 1, o)

    accd = [None] * NT

    def d_work(i):
        for r0, nr, c0, nc in _rects(D, *units_d[i][0]):
            oc = ocol[r0 // _CH // _DSTEP, pl.ds(r0 % _CH, nr), :].reshape(nr // 8, 8, 128)
            for c in range(c0, c0 + nc, 128):
                w = wo_v[r0:r0 + nr, c:c + 128].astype(_F32).reshape(nr // 8, 8, 128)
                part = jnp.sum(w * oc, axis=0)
                accd[c // 128] = part if accd[c // 128] is None else accd[c // 128] + part

    o = None
    done = 0
    for i in range(len(units_d)):
        for p in units_d[i][1]:
            piece(p, d_sems.at[i]).wait()
        d_issue(i + 1 + _AHEAD, i + 1 + _DEF_HI_AHEAD)
        if i in (0, 4):
            for s in range(i // 4 * _STEPS // 2, (i // 4 + 1) * _STEPS // 2):
                o = v_step(NCH - 1, s, o)
        if i == 8:
            v_finish(NCH - 1, o)
            x = jnp.broadcast_to(x_v[0].astype(_F32), (8, D))
            ga = mod_v[:, 2 * D:3 * D]
            f = 1.0 + mod_v[:, 4 * D:5 * D]
            g = gsh[...]
            sf, sg, sff, sfg, sgg = [_mean(t) for t in (f, g, f * f, f * g, g * g)]
        if i >= 10:
            while done <= i:
                d_work(done)
                done += 1
        if i == 12:
            base = acc[...]
            xs = x - _mean(x + ga * _allsum8(base + jnp.concatenate(accd, axis=1)))

    ga_attn = ga * _allsum8(base + jnp.concatenate(accd, axis=1))
    x1 = x + ga_attn
    a = xs + ga_attn
    e = a * f
    sa, saa, se, see, sef, seg = [_mean(t) for t in (a, a * a, e, e * e, e * f, e * g)]
    r = jax.lax.rsqrt(jnp.maximum(saa - sa * sa, 0.0) + _EPS)
    m2 = r * (se - sa * sf) + sg
    ms2 = r * (r * (see - sa * (2.0 * sef - sa * sff)) + 2.0 * (seg - sa * sfg)) + sgg
    r2 = jax.lax.rsqrt(jnp.maximum(ms2 - m2 * m2, 0.0) + _EPS)
    h3 = ((e - sa * f) * r + (g - m2)) * r2

    ys = [None] * NT
    gb = [None] * NT

    def tanh_tile(i, ht):
        v = (w1b[i * 128:(i + 1) * 128, :].reshape(16, 8, 128) * ht
             + b1b[i * 128:(i + 1) * 128, :].reshape(16, 8, 128))
        return jnp.tanh(v * (v * v + k0 / alpha)).reshape(128, 128)

    def reduce_tile(i, t, th):
        part = jnp.dot(ab_v[:, i * 128:(i + 1) * 128].astype(th.dtype), th, preferred_element_type=_F32)
        ys[t] = part if ys[t] is None else part + ys[t]

    def gate_tile(t, r0):
        part = jnp.dot(sc_v[:, r0:r0 + 128].astype(_BF16),
                       wm_v[r0:r0 + 128, 5 * D + t * 128:5 * D + (t + 1) * 128], preferred_element_type=_F32)
        gb[t] = part + gb[t]

    for i in range(NB - 2):
        older = list(ys)
        for t in range(NT):
            reduce_tile(i, t, tanh_tile(i, h3[:, t * 128:(t + 1) * 128]))
    for t in range(NT):
        ht = jnp.where(older[t] > inf_v[...], 0.0, h3[:, t * 128:(t + 1) * 128])
        th_v[:, t * 128:(t + 1) * 128] = tanh_tile(NB - 2, ht)

    gb_cp.wait()
    n = D - _GB_MXU
    for t in range(NT):
        w = wm_v[_GB_MXU:D, 5 * D + t * 128:5 * D + (t + 1) * 128].astype(_F32)
        p3 = (w * scb[...]).reshape(n // 8, 8, 128)
        gb[t] = _allsum8(jnp.sum(p3[:n // 16] + p3[n // 16:], axis=0))
    pending = [functools.partial(lambda t: reduce_tile(
        NB - 2, t, th_v[:, t * 128:(t + 1) * 128].astype(_BF16)), t) for t in range(NT)]
    pending += [functools.partial(gate_tile, t, r0) for r0 in range(0, _GB_MXU, 128) for t in range(NT)]
    per = -(-len(pending) // NT)
    for t in range(NT):
        for fn in pending[t * per:(t + 1) * per]:
            fn()
        reduce_tile(NB - 1, t, tanh_tile(NB - 1, h3[:, t * 128:(t + 1) * 128]))

    lin = lin_v[...]
    outs = []
    for t in range(NT):
        yy = ys[t] + lin
        y = h3[0:1, t * 128:(t + 1) * 128] * (yy[0:1] + yy[1:2]) + (yy[2:3] + yy[3:4])
        outs.append(x1[0:1, t * 128:(t + 1) * 128] + gb[t][0:1] * y)
    o_ref[0] = jnp.concatenate(outs, axis=1).astype(o_ref.dtype)


@jax.jit
def pallas_adaLN_cond__sliding_block_cached__mixer_token_mlp__decode_kernel(
    A_x: jax.Array,
    A_k_cache: jax.Array,
    A_v_cache: jax.Array,
    A_wq: jax.Array,
    A_wo: jax.Array,
    B_x: jax.Array,
    B_w1: jax.Array,
    B_b1: jax.Array,
    B_w2: jax.Array,
    B_b2: jax.Array,
    c: jax.Array,
    w_mod: jax.Array,
):
    B, Sq, D = A_x.shape
    _, H, Sk, Dh = A_k_cache.shape
    F = B_w1.shape[1]
    assert B == 1 and Sq == 1 and B_w1.shape[0] == 1
    W = min(4096, max(256, Sk // 4))
    HD = H * Dh
    assert A_wq.shape == (D, HD) and W == 4096

    kt = jnp.swapaxes(A_k_cache, 2, 3).reshape(HD, Sk)
    vt = jnp.swapaxes(A_v_cache, 2, 3).reshape(HD, Sk)
    b1 = B_b1.reshape(F // 128, 128)
    w2 = B_w2.reshape(1, F)
    b2 = B_b2.reshape(1, 1)

    NG = H // _GROUP
    scratch = [
        pltpu.VMEM((1, 1, D), _BF16),
        pltpu.VMEM((1, D), _BF16),
        pltpu.VMEM((1, F), _BF16),
        pltpu.VMEM((F // 128, 128), _BF16),
        pltpu.VMEM((1, F), _BF16),
        pltpu.VMEM((1, 1), _BF16),
        pltpu.VMEM((D, 6 * D), _BF16),
        pltpu.VMEM((D, HD), _BF16),
        pltpu.VMEM((HD, D), _BF16),
        pltpu.VMEM((_RING, _CH, W), _BF16),
        pltpu.VMEM((2, _GROUP, _CH), _F32),
        pltpu.VMEM((NG, _GROUP, W), _F32),
        pltpu.VMEM((NG, _GROUP, W), _F32),
        pltpu.VMEM((NG, _GROUP, 128), _F32),
        pltpu.VMEM((_GROUP, D), _F32),
        pltpu.VMEM((8, 5 * D), _F32),
        pltpu.VMEM((8, D), _F32),
        pltpu.VMEM((8, D), _F32),
        pltpu.VMEM((F, 128), _F32),
        pltpu.VMEM((F, 128), _F32),
        pltpu.VMEM((8, F), _F32),
        pltpu.VMEM((8, 128), _F32),
        pltpu.VMEM((D - _GB_MXU, 128), _F32),
        pltpu.VMEM((_NDEF, _CH, 128), _F32),
        pltpu.VMEM((8, D), _F32),
        pltpu.VMEM((128, D), _F32),
        pltpu.VMEM((8, 128), _F32),
        pltpu.SemaphoreType.DMA((6,)),
        pltpu.SemaphoreType.DMA((_AHEAD,)),
        pltpu.SemaphoreType.DMA((2 * _NU,)),
        pltpu.SemaphoreType.DMA((1,)),
        pltpu.SemaphoreType.DMA((3 * _NDEF,)),
    ]
    return pl.pallas_call(
        functools.partial(_kernel, D=D, H=H, Dh=Dh, Sk=Sk, W=W, F=F),
        out_shape=jax.ShapeDtypeStruct(A_x.shape, A_x.dtype),
        in_specs=[pl.BlockSpec(memory_space=pl.ANY)] * 11,
        out_specs=pl.BlockSpec(memory_space=pltpu.VMEM),
        scratch_shapes=scratch,
        compiler_params=pltpu.CompilerParams(
            vmem_limit_bytes=64 * 1024 * 1024,
            disable_bounds_checks=True,
            disable_semaphore_checks=True),
    )(A_x, kt, vt, A_wq, A_wo, B_w1, b1, w2, b2, c, w_mod)
```

```python
import functools
import math

import jax
import jax.numpy as jnp
import jax.experimental.pallas as pl
import jax.experimental.pallas.tpu as pltpu

_F32 = jnp.float32
_BF16 = jnp.bfloat16

_EPS = 1e-05
_GROUP = 8
_CH = 128
_RING = 4
_UR = 8
_NU = _CH // _UR
_AHEAD = 20
_LAG = 4
_PA, _PP = 1792, 384
_STEPS = 4
_WIN = 32
_WIN_HI = 3
_OFF_W, _OFF_M = 17, 28
_NDEF, _DSTEP = 8, 4
_DEF_HI_AHEAD = 16
_GB_MXU = 384


def _rects(ncols, t0, t1):
    tpr = ncols // 128
    out = []
    while t0 < t1:
        g, c = divmod(t0, tpr)
        if c == 0 and t1 - t0 >= tpr:
            n = (t1 - t0) // tpr
            out.append((g * 8, n * 8, 0, ncols))
            t0 += n * tpr
        else:
            e = min(tpr, c + (t1 - t0))
            out.append((g * 8, 8, c * 128, (e - c) * 128))
            t0 += e - c
    return out


def _unit(src, dst, ncols, cmax, spans):
    tiles = [t for a, b in spans for t in range(a, b) if (t % (ncols // 128)) * 128 < cmax]
    n_hi = _WIN_HI if len(tiles) > 2 * _WIN_HI else 0
    pieces = []
    for part, prio in ((tiles[:len(tiles) - n_hi], 1), (tiles[len(tiles) - n_hi:], 0)):
        i = 0
        while i < len(part):
            k = i
            while k + 1 < len(part) and part[k + 1] == part[k] + 1:
                k += 1
            pieces += [(src, dst) + r + (prio,) for r in _rects(ncols, part[i], part[k] + 1)]
            i = k + 1
    return pieces


def _windows(src, dst, shape, off, cmax, skip=()):
    nt = shape[0] // 8 * (shape[1] // 128)
    starts = list(range(off - _WIN, nt, _WIN))
    out = []
    for b in range(8):
        for s in starts[b::8]:
            spans = [(max(s, 0), min(s + _WIN, nt))]
            for h0, h1 in skip:
                spans = [x for p, q in spans for x in ((p, min(q, h0)), (max(p, h1), q)) if x[0] < x[1]]
            u = _unit(src, dst, shape[1], cmax, spans)
            if u:
                out.append(u)
    return out


def _interleave(*lists):
    items = sorted(((k + 0.5) / len(p), n, k) for n, p in enumerate(lists) for k in range(len(p)))
    return [lists[n][k] for _, n, k in items]


def _mean(v):
    return jnp.sum(v, axis=-1, keepdims=True) * (1.0 / v.shape[-1])


def _layernorm(v):
    d = v - _mean(v)
    return d * jax.lax.rsqrt(_mean(d * d) + _EPS)


def _allsum8(v):
    v = v + pltpu.roll(v, 4, 0)
    v = v + pltpu.roll(v, 2, 0)
    return v + pltpu.roll(v, 1, 0)


def _columns(row):
    return jnp.broadcast_to(row, (128, 128)).T


def _aligned(i, n):
    return i if isinstance(i, int) else pl.multiple_of(i, n)


def _kernel(
    x_hbm, k_hbm, v_hbm, wq_hbm, wo_hbm, w1_hbm, b1_hbm, w2_hbm, b2_hbm, c_hbm, wm_hbm,
    o_ref,
    x_v, c_v, w1_v, b1_v, w2_v, b2_v, wm_v, wq_v, wo_v, ring, qbd, s_acc, p_buf, linv, acc,
    mod_v, h_v, sc_v, w1b, b1b, ab_v, lin_v, scb, ocol, gsh, th_v, inf_v,
    small_sems, w_sems, kv_sems, g_sem, d_sems,
    *, D, H, Dh, Sk, W, F,
):
    HD = H * Dh
    NG = H // _GROUP
    NCH = HD // _CH
    CPG = _GROUP * Dh // _CH
    CW = W // _STEPS
    TPS = _NU // _STEPS
    NT = D // 128
    NB = F // 128
    scale = Dh ** (-0.5)
    k0 = math.sqrt(2.0 / math.pi)
    alpha = (k0 * 0.044715) ** (1.0 / 3.0)

    def kv_piece(src, j, c, u, c0, nc):
        r = _aligned(j * _CH + u * _UR, _UR)
        return pltpu.make_async_copy(
            src.at[pl.ds(r, _UR), pl.ds(Sk - W + c0, nc)],
            ring.at[c % _RING, pl.ds(u * _UR, _UR), pl.ds(c0, nc)],
            kv_sems.at[(c % 2) * _NU + u])

    def kv_issue(where, c, u):
        dc, uu = divmod(u, _NU)
        t = where(dc)
        if t is not None:
            kv_piece(t[0], t[1], c + dc, uu, 0, _PA).start(priority=1)
            kv_piece(t[0], t[1], c + dc, uu, _PA, _PP).start(priority=0)
        dc, uu = divmod(u - _LAG, _NU)
        t = where(dc) if dc >= 0 else None
        if t is not None:
            kv_piece(t[0], t[1], c + dc, uu, _PA + _PP, W - _PA - _PP).start(priority=1)

    def where_static(c):
        def where(dc):
            if c + dc < NCH:
                return (k_hbm, c + dc)
            if c + dc < 2 * NCH:
                return (v_hbm, c + dc - NCH)
            return None
        return where

    def tick(where, c, u):
        kv_piece(k_hbm, 0, c, u, 0, W).wait()
        kv_issue(where, c, u + _AHEAD)

    tpc = _CH // 8 * NT
    holes = [(j * _DSTEP * tpc, (j * _DSTEP + 1) * tpc) for j in range(_NDEF)]
    units_mq = _interleave(_windows(wm_hbm, wm_v, (D, 6 * D), _OFF_M, 5 * D),
                           _windows(wq_hbm, wq_v, (D, HD), _OFF_W, HD))
    pre = units_mq + _windows(wo_hbm, wo_v, (HD, D), _OFF_W, D, holes)
    units_d = []
    for p in (1, 2, 0):
        for h0, h1 in holes:
            cuts = [h0] + [t for t in range(h0 + 1, h1) if t % _WIN == _OFF_W] + [h1]
            assert len(cuts) == 4
            span = (cuts[p], cuts[p + 1])
            units_d.append((span, _unit(wo_hbm, wo_v, D, D, [span])))

    def piece(p, sem):
        src, dst, r0, nr, c0, nc, _ = p
        return pltpu.make_async_copy(
            src.at[pl.ds(r0, nr), pl.ds(c0, nc)], dst.at[pl.ds(r0, nr), pl.ds(c0, nc)], sem)

    def w_start(i):
        for p in pre[i]:
            piece(p, w_sems.at[i % _AHEAD]).start(priority=p[-1])

    def w_wait(i):
        for p in pre[i]:
            piece(p, w_sems.at[i % _AHEAD]).wait()

    small = [(c_hbm, c_v), (x_hbm, x_v), (w1_hbm, w1_v), (b1_hbm, b1_v), (w2_hbm, w2_v), (b2_hbm, b2_v)]
    small_cp = [pltpu.make_async_copy(s, d, small_sems.at[i]) for i, (s, d) in enumerate(small)]
    gb_cp = pltpu.make_async_copy(
        wm_hbm.at[:, pl.ds(5 * D, D)], wm_v.at[:, pl.ds(5 * D, D)], g_sem.at[0])
    d_next = [0, 0]

    def d_issue(upto_lo, upto_hi):
        while d_next[0] < upto_lo:
            i = d_next[0]
            if i < len(units_d):
                for p in units_d[i][1]:
                    if p[-1] == 1:
                        piece(p, d_sems.at[i]).start(priority=1)
            elif i == len(units_d):
                gb_cp.start(priority=1)
            d_next[0] += 1
        while d_next[1] < min(upto_hi, len(units_d)):
            i = d_next[1]
            for p in units_d[i][1]:
                if p[-1] == 0:
                    piece(p, d_sems.at[i]).start(priority=0)
            d_next[1] += 1

    def prep_small():
        c = c_v[...].astype(_F32)
        sc = (c * jax.nn.sigmoid(c)).astype(_BF16).astype(_F32)
        sc_v[...] = jnp.broadcast_to(sc, (8, D))
        s_acc[...] = jnp.zeros(s_acc.shape, _F32)
        acc[...] = jnp.zeros(acc.shape, _F32)
        inf_v[...] = jnp.full(inf_v.shape, jnp.inf, _F32)

    def prep_scb(r):
        scb[r - _GB_MXU:r - _GB_MXU + 128, :] = _columns(sc_v[0:1, r:r + 128])

    def prep_mlp(i):
        w1 = w1_v[:, i * 128:(i + 1) * 128].astype(_F32)
        w2 = w2_v[:, i * 128:(i + 1) * 128].astype(_F32)
        b1 = b1_v[...].astype(_F32)[i:i + 1, :]
        w1b[i * 128:(i + 1) * 128, :] = _columns(w1 * alpha)
        b1b[i * 128:(i + 1) * 128, :] = _columns(b1 * alpha)
        a = 0.5 * w2 * w1
        b = 0.5 * w2 * b1
        a_hi = a.astype(_BF16).astype(_F32)
        b_hi = b.astype(_BF16).astype(_F32)
        sub = jax.lax.broadcasted_iota(jnp.int32, (8, 128), 0)
        ab_v[:, i * 128:(i + 1) * 128] = jnp.where(
            sub == 0, a_hi, jnp.where(sub == 1, a - a_hi, jnp.where(
                sub == 2, b_hi, jnp.where(sub == 3, b - b_hi, 0.0))))

    def prep_lin():
        sub = jax.lax.broadcasted_iota(jnp.int32, (8, 128), 0)
        tot = jnp.broadcast_to(jnp.sum(ab_v[...], axis=1, keepdims=True), (8, 128))
        lin_v[...] = tot + jnp.where(sub == 2, jnp.broadcast_to(b2_v[...].astype(_F32), (8, 128)), 0.0)

    def mod_tiles(t0, t1):
        mod_v[:, t0 * 128:t1 * 128] = jnp.dot(
            sc_v[...].astype(_BF16), wm_v[:, t0 * 128:t1 * 128], preferred_element_type=_F32)

    def make_h():
        x = jnp.broadcast_to(x_v[0].astype(_F32), (8, D))
        h_v[...] = _layernorm(x) * (1.0 + mod_v[:, D:2 * D]) + mod_v[:, 0:D]
        sb = mod_v[:, 3 * D:4 * D]
        gsh[...] = sb - _mean(sb)

    work = {}
    items = [prep_small] + [functools.partial(prep_scb, r) for r in range(_GB_MXU, D, 128)]
    items += [functools.partial(prep_mlp, i) for i in range(NB)] + [prep_lin]
    for k, fn in enumerate(items):
        work[12 + 6 * k] = fn
    assert 12 + 6 * len(items) <= len(units_mq)
    items = [functools.partial(mod_tiles, t, min(t + 2, 5 * NT)) for t in range(0, 5 * NT, 2)] + [make_h]
    for k, fn in enumerate(items):
        work[len(units_mq) + 5 * k] = fn
    assert len(units_mq) + 5 * len(items) <= len(pre)

    for i in range(_AHEAD):
        w_start(i)
    for cp in small_cp:
        cp.start()
    for i in range(len(pre)):
        w_wait(i)
        if i + _AHEAD < len(pre):
            w_start(i + _AHEAD)
        else:
            kv_issue(where_static(0), 0, i + _AHEAD - len(pre))
        if i == 8:
            for cp in small_cp:
                cp.wait()
        if i in work:
            work[i]()

    def diag_mask(j):
        lo = jax.lax.broadcasted_iota(jnp.int32, (_GROUP, _CH), 0) * Dh - (j % CPG) * _CH
        col = jax.lax.broadcasted_iota(jnp.int32, (_GROUP, _CH), 1)
        return (col >= lo) & (col < lo + Dh)

    def q_tile(j):
        q = jnp.dot(h_v[...].astype(_BF16), wq_v[:, pl.ds(_aligned(j * _CH, _CH), _CH)],
                    preferred_element_type=_F32)
        qbd[j % 2] = jnp.where(diag_mask(j), q, 0.0)

    def k_step(j, s):
        cols = pl.ds(s * CW, CW)
        s_acc[j // CPG, :, cols] += jnp.dot(
            qbd[j % 2].astype(_BF16), ring[j % _RING, :, cols], preferred_element_type=_F32)

    def softmax(g):
        s = s_acc[g]
        m = jnp.max(s, axis=-1, keepdims=True)
        p = jnp.exp((s - m) * scale)
        p_buf[g] = p
        linv[g] = jnp.broadcast_to(1.0 / jnp.sum(p, axis=-1, keepdims=True), (_GROUP, 128))

    def v_step(j, s, o):
        cols = pl.ds(s * CW, CW)
        part = jax.lax.dot_general(
            p_buf[j // CPG, :, cols].astype(_BF16), ring[(j + NCH) % _RING, :, cols],
            (((1,), (1,)), ((), ())), preferred_element_type=_F32)
        return part if o is None else part + o

    def v_finish(j, o):
        o = jnp.where(diag_mask(j), o * linv[j // CPG], 0.0).astype(_BF16)

        def now():
            acc[...] += jnp.dot(o, wo_v[pl.ds(_aligned(j * _CH, _CH), _CH), :], preferred_element_type=_F32)

        def later():
            ocol[j // _DSTEP] = _columns(jnp.sum(o.astype(_F32), axis=0, keepdims=True))

        if isinstance(j, int):
            assert j >= _DSTEP * _NDEF
            now()
        else:
            deferred = jnp.logical_and(j % _DSTEP == 0, j < _DSTEP * _NDEF)
            pl.when(deferred)(later)
            pl.when(jnp.logical_not(deferred))(now)

    def k_chunk(where, c, first=False, last=False):
        for u in range(_NU):
            tick(where, c, u)
            if u % TPS == 0 and not first:
                k_step(c - 1, u // TPS)
            if u == _NU - 2 and not last:
                q_tile(c)

    def k_body(c, carry):
        k_chunk(lambda dc: (k_hbm, c + dc), c)

        @pl.when(c % CPG == 0)
        def _():
            softmax(c // CPG - 1)
        return carry

    k_chunk(where_static(0), 0, first=True)
    jax.lax.fori_loop(1, NCH - 2, k_body, 0)
    for c in range(NCH - 2, NCH + 1):
        k_chunk(where_static(c), c, last=c == NCH)
    softmax(NG - 1)

    def v_body(j, carry):
        o = None
        for u in range(_NU):
            tick(lambda dc: (v_hbm, j + dc), NCH + j, u)
            if u % TPS == 0:
                o = v_step(j - 1, u // TPS, o)
        v_finish(j - 1, o)
        return carry

    jax.lax.fori_loop(1, NCH - 2, v_body, 0)
    nleft = _AHEAD - _LAG + 1
    for j in range(NCH - 2, NCH):
        o = None
        for u in range(_NU):
            tick(where_static(NCH + j), NCH + j, u)
            k = nleft - ((NCH - j) * _NU - u) + 1
            if k > 0:
                d_issue(k * _AHEAD // nleft, k * _DEF_HI_AHEAD // nleft)
            if u % TPS == 0:
                o = v_step(j - 1, u // TPS, o)
        v_finish(j - 1, o)

    accd = [None] * NT

    def d_work(i):
        for r0, nr, c0, nc in _rects(D, *units_d[i][0]):
            oc = ocol[r0 // _CH // _DSTEP, pl.ds(r0 % _CH, nr), :].reshape(nr // 8, 8, 128)
            for c in range(c0, c0 + nc, 128):
                w = wo_v[r0:r0 + nr, c:c + 128].astype(_F32).reshape(nr // 8, 8, 128)
                part = jnp.sum(w * oc, axis=0)
                accd[c // 128] = part if accd[c // 128] is None else accd[c // 128] + part

    o = None
    done = 0
    for i in range(len(units_d)):
        for p in units_d[i][1]:
            piece(p, d_sems.at[i]).wait()
        d_issue(i + 1 + _AHEAD, i + 1 + _DEF_HI_AHEAD)
        if i in (0, 4):
            for s in range(i // 4 * _STEPS // 2, (i // 4 + 1) * _STEPS // 2):
                o = v_step(NCH - 1, s, o)
        if i == 8:
            v_finish(NCH - 1, o)
            x = jnp.broadcast_to(x_v[0].astype(_F32), (8, D))
            ga = mod_v[:, 2 * D:3 * D]
            f = 1.0 + mod_v[:, 4 * D:5 * D]
            g = gsh[...]
            sf, sg, sff, sfg, sgg = [_mean(t) for t in (f, g, f * f, f * g, g * g)]
        if i >= 10:
            while done <= i:
                d_work(done)
                done += 1
        if i == 12:
            base = acc[...]
            x1 = x + ga * _allsum8(base + jnp.concatenate(accd, axis=1))
            m1 = _mean(x1)
        if i == 14:
            r1 = jax.lax.rsqrt(_mean((x1 - m1) * (x1 - m1)) + _EPS)
            xs = (x - m1) * r1
            gs = ga * r1
            eps1 = _EPS * r1 * r1

    attn = _allsum8(base + jnp.concatenate(accd, axis=1))
    x1 = x + ga * attn
    a = xs + gs * attn
    e = a * f
    sa, saa, se, see, sef, seg = [_mean(t) for t in (a, a * a, e, e * e, e * f, e * g)]
    r = jax.lax.rsqrt(jnp.maximum(saa - sa * sa, 0.0) + eps1)
    m2 = r * (se - sa * sf) + sg
    ms2 = r * (r * (see - sa * (2.0 * sef - sa * sff)) + 2.0 * (seg - sa * sfg)) + sgg
    r2 = jax.lax.rsqrt(jnp.maximum(ms2 - m2 * m2, 0.0) + _EPS)
    h3 = ((e - sa * f) * r + (g - m2)) * r2

    ys = [None] * NT
    gb = [None] * NT

    def tanh_tile(i, ht):
        v = (w1b[i * 128:(i + 1) * 128, :].reshape(16, 8, 128) * ht
             + b1b[i * 128:(i + 1) * 128, :].reshape(16, 8, 128))
        return jnp.tanh(v * (v * v + k0 / alpha)).reshape(128, 128)

    def reduce_tile(i, t, th):
        part = jnp.dot(ab_v[:, i * 128:(i + 1) * 128].astype(th.dtype), th, preferred_element_type=_F32)
        ys[t] = part if ys[t] is None else part + ys[t]

    def gate_tile(t, r0):
        part = jnp.dot(sc_v[:, r0:r0 + 128].astype(_BF16),
                       wm_v[r0:r0 + 128, 5 * D + t * 128:5 * D + (t + 1) * 128], preferred_element_type=_F32)
        gb[t] = part + gb[t]

    for i in range(NB - 2):
        older = list(ys)
        for t in range(NT):
            reduce_tile(i, t, tanh_tile(i, h3[:, t * 128:(t + 1) * 128]))
    for t in range(NT):
        ht = jnp.where(older[t] > inf_v[...], 0.0, h3[:, t * 128:(t + 1) * 128])
        th_v[:, t * 128:(t + 1) * 128] = tanh_tile(NB - 2, ht)

    gb_cp.wait()
    n = D - _GB_MXU
    for t in range(NT):
        w = wm_v[_GB_MXU:D, 5 * D + t * 128:5 * D + (t + 1) * 128].astype(_F32)
        p3 = (w * scb[...]).reshape(n // 8, 8, 128)
        gb[t] = _allsum8(jnp.sum(p3[:n // 16] + p3[n // 16:], axis=0))
    pending = [functools.partial(lambda t: reduce_tile(
        NB - 2, t, th_v[:, t * 128:(t + 1) * 128].astype(_BF16)), t) for t in range(NT)]
    pending += [functools.partial(gate_tile, t, r0) for r0 in range(0, _GB_MXU, 128) for t in range(NT)]
    per = -(-len(pending) // NT)
    for t in range(NT):
        for fn in pending[t * per:(t + 1) * per]:
            fn()
        reduce_tile(NB - 1, t, tanh_tile(NB - 1, h3[:, t * 128:(t + 1) * 128]))

    lin = lin_v[...]
    outs = []
    for t in range(NT):
        yy = ys[t] + lin
        y = h3[0:1, t * 128:(t + 1) * 128] * (yy[0:1] + yy[1:2]) + (yy[2:3] + yy[3:4])
        outs.append(x1[0:1, t * 128:(t + 1) * 128] + gb[t][0:1] * y)
    o_ref[0] = jnp.concatenate(outs, axis=1).astype(o_ref.dtype)


@jax.jit
def pallas_adaLN_cond__sliding_block_cached__mixer_token_mlp__decode_kernel(
    A_x: jax.Array,
    A_k_cache: jax.Array,
    A_v_cache: jax.Array,
    A_wq: jax.Array,
    A_wo: jax.Array,
    B_x: jax.Array,
    B_w1: jax.Array,
    B_b1: jax.Array,
    B_w2: jax.Array,
    B_b2: jax.Array,
    c: jax.Array,
    w_mod: jax.Array,
):
    B, Sq, D = A_x.shape
    _, H, Sk, Dh = A_k_cache.shape
    F = B_w1.shape[1]
    assert B == 1 and Sq == 1 and B_w1.shape[0] == 1
    W = min(4096, max(256, Sk // 4))
    HD = H * Dh
    assert A_wq.shape == (D, HD) and W == 4096

    kt = jnp.swapaxes(A_k_cache, 2, 3).reshape(HD, Sk)
    vt = jnp.swapaxes(A_v_cache, 2, 3).reshape(HD, Sk)
    b1 = B_b1.reshape(F // 128, 128)
    w2 = B_w2.reshape(1, F)
    b2 = B_b2.reshape(1, 1)

    NG = H // _GROUP
    scratch = [
        pltpu.VMEM((1, 1, D), _BF16),
        pltpu.VMEM((1, D), _BF16),
        pltpu.VMEM((1, F), _BF16),
        pltpu.VMEM((F // 128, 128), _BF16),
        pltpu.VMEM((1, F), _BF16),
        pltpu.VMEM((1, 1), _BF16),
        pltpu.VMEM((D, 6 * D), _BF16),
        pltpu.VMEM((D, HD), _BF16),
        pltpu.VMEM((HD, D), _BF16),
        pltpu.VMEM((_RING, _CH, W), _BF16),
        pltpu.VMEM((2, _GROUP, _CH), _F32),
        pltpu.VMEM((NG, _GROUP, W), _F32),
        pltpu.VMEM((NG, _GROUP, W), _F32),
        pltpu.VMEM((NG, _GROUP, 128), _F32),
        pltpu.VMEM((_GROUP, D), _F32),
        pltpu.VMEM((8, 5 * D), _F32),
        pltpu.VMEM((8, D), _F32),
        pltpu.VMEM((8, D), _F32),
        pltpu.VMEM((F, 128), _F32),
        pltpu.VMEM((F, 128), _F32),
        pltpu.VMEM((8, F), _F32),
        pltpu.VMEM((8, 128), _F32),
        pltpu.VMEM((D - _GB_MXU, 128), _F32),
        pltpu.VMEM((_NDEF, _CH, 128), _F32),
        pltpu.VMEM((8, D), _F32),
        pltpu.VMEM((128, D), _F32),
        pltpu.VMEM((8, 128), _F32),
        pltpu.SemaphoreType.DMA((6,)),
        pltpu.SemaphoreType.DMA((_AHEAD,)),
        pltpu.SemaphoreType.DMA((2 * _NU,)),
        pltpu.SemaphoreType.DMA((1,)),
        pltpu.SemaphoreType.DMA((3 * _NDEF,)),
    ]
    return pl.pallas_call(
        functools.partial(_kernel, D=D, H=H, Dh=Dh, Sk=Sk, W=W, F=F),
        out_shape=jax.ShapeDtypeStruct(A_x.shape, A_x.dtype),
        in_specs=[pl.BlockSpec(memory_space=pl.ANY)] * 11,
        out_specs=pl.BlockSpec(memory_space=pltpu.VMEM),
        scratch_shapes=scratch,
        compiler_params=pltpu.CompilerParams(
            vmem_limit_bytes=64 * 1024 * 1024,
            disable_bounds_checks=True,
            disable_semaphore_checks=True),
    )(A_x, kt, vt, A_wq, A_wo, B_w1, b1, w2, b2, c, w_mod)
```

```python
import functools
import math

import jax
import jax.numpy as jnp
import jax.experimental.pallas as pl
import jax.experimental.pallas.tpu as pltpu

_F32 = jnp.float32
_BF16 = jnp.bfloat16

_EPS = 1e-05
_GROUP = 8
_CH = 128
_RING = 4
_UR = 8
_NU = _CH // _UR
_AHEAD = 21
_LAG = 5
_PA, _PP = 1792, 384
_STEPS = 4
_WIN = 32
_WIN_HI = 3
_OFF_W, _OFF_M = 17, 28
_NDEF, _DSTEP = 8, 4
_DEF_HI_AHEAD = 16
_GB_MXU = 384


def _rects(ncols, t0, t1):
    tpr = ncols // 128
    out = []
    while t0 < t1:
        g, c = divmod(t0, tpr)
        if c == 0 and t1 - t0 >= tpr:
            n = (t1 - t0) // tpr
            out.append((g * 8, n * 8, 0, ncols))
            t0 += n * tpr
        else:
            e = min(tpr, c + (t1 - t0))
            out.append((g * 8, 8, c * 128, (e - c) * 128))
            t0 += e - c
    return out


def _unit(src, dst, ncols, cmax, spans):
    tiles = [t for a, b in spans for t in range(a, b) if (t % (ncols // 128)) * 128 < cmax]
    n_hi = _WIN_HI if len(tiles) > 2 * _WIN_HI else 0
    pieces = []
    for part, prio in ((tiles[:len(tiles) - n_hi], 1), (tiles[len(tiles) - n_hi:], 0)):
        i = 0
        while i < len(part):
            k = i
            while k + 1 < len(part) and part[k + 1] == part[k] + 1:
                k += 1
            pieces += [(src, dst) + r + (prio,) for r in _rects(ncols, part[i], part[k] + 1)]
            i = k + 1
    return pieces


def _windows(src, dst, shape, off, cmax, skip=()):
    nt = shape[0] // 8 * (shape[1] // 128)
    starts = list(range(off - _WIN, nt, _WIN))
    out = []
    for b in range(8):
        for s in starts[b::8]:
            spans = [(max(s, 0), min(s + _WIN, nt))]
            for h0, h1 in skip:
                spans = [x for p, q in spans for x in ((p, min(q, h0)), (max(p, h1), q)) if x[0] < x[1]]
            u = _unit(src, dst, shape[1], cmax, spans)
            if u:
                out.append(u)
    return out


def _interleave(*lists):
    items = sorted(((k + 0.5) / len(p), n, k) for n, p in enumerate(lists) for k in range(len(p)))
    return [lists[n][k] for _, n, k in items]


def _mean(v):
    return jnp.sum(v, axis=-1, keepdims=True) * (1.0 / v.shape[-1])


def _layernorm(v):
    d = v - _mean(v)
    return d * jax.lax.rsqrt(_mean(d * d) + _EPS)


def _allsum8(v):
    v = v + pltpu.roll(v, 4, 0)
    v = v + pltpu.roll(v, 2, 0)
    return v + pltpu.roll(v, 1, 0)


def _columns(row):
    return jnp.broadcast_to(row, (128, 128)).T


def _aligned(i, n):
    return i if isinstance(i, int) else pl.multiple_of(i, n)


def _kernel(
    x_hbm, k_hbm, v_hbm, wq_hbm, wo_hbm, w1_hbm, b1_hbm, w2_hbm, b2_hbm, c_hbm, wm_hbm,
    o_ref,
    x_v, c_v, w1_v, b1_v, w2_v, b2_v, wm_v, wq_v, wo_v, ring, qbd, s_acc, p_buf, linv, acc,
    mod_v, h_v, sc_v, w1b, b1b, ab_v, lin_v, scb, ocol, gsh, th_v, inf_v,
    small_sems, w_sems, kv_sems, g_sem, d_sems,
    *, D, H, Dh, Sk, W, F,
):
    HD = H * Dh
    NG = H // _GROUP
    NCH = HD // _CH
    CPG = _GROUP * Dh // _CH
    CW = W // _STEPS
    TPS = _NU // _STEPS
    NT = D // 128
    NB = F // 128
    scale = Dh ** (-0.5)
    k0 = math.sqrt(2.0 / math.pi)
    alpha = (k0 * 0.044715) ** (1.0 / 3.0)

    def kv_piece(src, j, c, u, c0, nc):
        r = _aligned(j * _CH + u * _UR, _UR)
        return pltpu.make_async_copy(
            src.at[pl.ds(r, _UR), pl.ds(Sk - W + c0, nc)],
            ring.at[c % _RING, pl.ds(u * _UR, _UR), pl.ds(c0, nc)],
            kv_sems.at[(c % 2) * _NU + u])

    def kv_issue(where, c, u):
        dc, uu = divmod(u, _NU)
        t = where(dc)
        if t is not None:
            kv_piece(t[0], t[1], c + dc, uu, 0, _PA).start(priority=1)
            kv_piece(t[0], t[1], c + dc, uu, _PA, _PP).start(priority=0)
        dc, uu = divmod(u - _LAG, _NU)
        t = where(dc) if dc >= 0 else None
        if t is not None:
            kv_piece(t[0], t[1], c + dc, uu, _PA + _PP, W - _PA - _PP).start(priority=1)

    def where_static(c):
        def where(dc):
            if c + dc < NCH:
                return (k_hbm, c + dc)
            if c + dc < 2 * NCH:
                return (v_hbm, c + dc - NCH)
            return None
        return where

    def tick(where, c, u):
        kv_piece(k_hbm, 0, c, u, 0, W).wait()
        kv_issue(where, c, u + _AHEAD)

    tpc = _CH // 8 * NT
    holes = [(j * _DSTEP * tpc, (j * _DSTEP + 1) * tpc) for j in range(_NDEF)]
    units_mq = _interleave(_windows(wm_hbm, wm_v, (D, 6 * D), _OFF_M, 5 * D),
                           _windows(wq_hbm, wq_v, (D, HD), _OFF_W, HD))
    pre = units_mq + _windows(wo_hbm, wo_v, (HD, D), _OFF_W, D, holes)
    units_d = []
    for p in (1, 2, 0):
        for h0, h1 in holes:
            cuts = [h0] + [t for t in range(h0 + 1, h1) if t % _WIN == _OFF_W] + [h1]
            assert len(cuts) == 4
            span = (cuts[p], cuts[p + 1])
            units_d.append((span, _unit(wo_hbm, wo_v, D, D, [span])))

    def piece(p, sem):
        src, dst, r0, nr, c0, nc, _ = p
        return pltpu.make_async_copy(
            src.at[pl.ds(r0, nr), pl.ds(c0, nc)], dst.at[pl.ds(r0, nr), pl.ds(c0, nc)], sem)

    def w_start(i):
        for p in pre[i]:
            piece(p, w_sems.at[i % _AHEAD]).start(priority=p[-1])

    def w_wait(i):
        for p in pre[i]:
            piece(p, w_sems.at[i % _AHEAD]).wait()

    small = [(c_hbm, c_v), (x_hbm, x_v), (w1_hbm, w1_v), (b1_hbm, b1_v), (w2_hbm, w2_v), (b2_hbm, b2_v)]
    small_cp = [pltpu.make_async_copy(s, d, small_sems.at[i]) for i, (s, d) in enumerate(small)]
    gb_cp = pltpu.make_async_copy(
        wm_hbm.at[:, pl.ds(5 * D, D)], wm_v.at[:, pl.ds(5 * D, D)], g_sem.at[0])
    d_next = [0, 0]

    def d_issue(upto_lo, upto_hi):
        while d_next[0] < upto_lo:
            i = d_next[0]
            if i < len(units_d):
                for p in units_d[i][1]:
                    if p[-1] == 1:
                        piece(p, d_sems.at[i]).start(priority=1)
            elif i == len(units_d):
                gb_cp.start(priority=1)
            d_next[0] += 1
        while d_next[1] < min(upto_hi, len(units_d)):
            i = d_next[1]
            for p in units_d[i][1]:
                if p[-1] == 0:
                    piece(p, d_sems.at[i]).start(priority=0)
            d_next[1] += 1

    def prep_small():
        c = c_v[...].astype(_F32)
        sc = (c * jax.nn.sigmoid(c)).astype(_BF16).astype(_F32)
        sc_v[...] = jnp.broadcast_to(sc, (8, D))
        s_acc[...] = jnp.zeros(s_acc.shape, _F32)
        acc[...] = jnp.zeros(acc.shape, _F32)
        inf_v[...] = jnp.full(inf_v.shape, jnp.inf, _F32)

    def prep_scb(r):
        scb[r - _GB_MXU:r - _GB_MXU + 128, :] = _columns(sc_v[0:1, r:r + 128])

    def prep_mlp(i):
        w1 = w1_v[:, i * 128:(i + 1) * 128].astype(_F32)
        w2 = w2_v[:, i * 128:(i + 1) * 128].astype(_F32)
        b1 = b1_v[...].astype(_F32)[i:i + 1, :]
        w1b[i * 128:(i + 1) * 128, :] = _columns(w1 * alpha)
        b1b[i * 128:(i + 1) * 128, :] = _columns(b1 * alpha)
        a = 0.5 * w2 * w1
        b = 0.5 * w2 * b1
        a_hi = a.astype(_BF16).astype(_F32)
        b_hi = b.astype(_BF16).astype(_F32)
        sub = jax.lax.broadcasted_iota(jnp.int32, (8, 128), 0)
        ab_v[:, i * 128:(i + 1) * 128] = jnp.where(
            sub == 0, a_hi, jnp.where(sub == 1, a - a_hi, jnp.where(
                sub == 2, b_hi, jnp.where(sub == 3, b - b_hi, 0.0))))

    def prep_lin():
        sub = jax.lax.broadcasted_iota(jnp.int32, (8, 128), 0)
        tot = jnp.broadcast_to(jnp.sum(ab_v[...], axis=1, keepdims=True), (8, 128))
        lin_v[...] = tot + jnp.where(sub == 2, jnp.broadcast_to(b2_v[...].astype(_F32), (8, 128)), 0.0)

    def mod_tiles(t0, t1):
        mod_v[:, t0 * 128:t1 * 128] = jnp.dot(
            sc_v[...].astype(_BF16), wm_v[:, t0 * 128:t1 * 128], preferred_element_type=_F32)

    def make_h():
        x = jnp.broadcast_to(x_v[0].astype(_F32), (8, D))
        h_v[...] = _layernorm(x) * (1.0 + mod_v[:, D:2 * D]) + mod_v[:, 0:D]
        sb = mod_v[:, 3 * D:4 * D]
        gsh[...] = sb - _mean(sb)

    work = {}
    items = [prep_small] + [functools.partial(prep_scb, r) for r in range(_GB_MXU, D, 128)]
    items += [functools.partial(prep_mlp, i) for i in range(NB)] + [prep_lin]
    for k, fn in enumerate(items):
        work[12 + 6 * k] = fn
    assert 12 + 6 * len(items) <= len(units_mq)
    items = [functools.partial(mod_tiles, t, min(t + 2, 5 * NT)) for t in range(0, 5 * NT, 2)] + [make_h]
    for k, fn in enumerate(items):
        work[len(units_mq) + 5 * k] = fn
    assert len(units_mq) + 5 * len(items) <= len(pre)

    for i in range(_AHEAD):
        w_start(i)
    for cp in small_cp:
        cp.start()
    for i in range(len(pre)):
        w_wait(i)
        if i + _AHEAD < len(pre):
            w_start(i + _AHEAD)
        else:
            kv_issue(where_static(0), 0, i + _AHEAD - len(pre))
        if i == 8:
            for cp in small_cp:
                cp.wait()
        if i in work:
            work[i]()

    def diag_mask(j):
        lo = jax.lax.broadcasted_iota(jnp.int32, (_GROUP, _CH), 0) * Dh - (j % CPG) * _CH
        col = jax.lax.broadcasted_iota(jnp.int32, (_GROUP, _CH), 1)
        return (col >= lo) & (col < lo + Dh)

    def q_tile(j):
        q = jnp.dot(h_v[...].astype(_BF16), wq_v[:, pl.ds(_aligned(j * _CH, _CH), _CH)],
                    preferred_element_type=_F32)
        qbd[j % 2] = jnp.where(diag_mask(j), q, 0.0)

    def k_step(j, s):
        cols = pl.ds(s * CW, CW)
        s_acc[j // CPG, :, cols] += jnp.dot(
            qbd[j % 2].astype(_BF16), ring[j % _RING, :, cols], preferred_element_type=_F32)

    def softmax(g):
        s = s_acc[g]
        m = jnp.max(s, axis=-1, keepdims=True)
        p = jnp.exp((s - m) * scale)
        p_buf[g] = p
        linv[g] = jnp.broadcast_to(1.0 / jnp.sum(p, axis=-1, keepdims=True), (_GROUP, 128))

    def v_step(j, s, o):
        cols = pl.ds(s * CW, CW)
        part = jax.lax.dot_general(
            p_buf[j // CPG, :, cols].astype(_BF16), ring[(j + NCH) % _RING, :, cols],
            (((1,), (1,)), ((), ())), preferred_element_type=_F32)
        return part if o is None else part + o

    def v_finish(j, o):
        o = jnp.where(diag_mask(j), o * linv[j // CPG], 0.0).astype(_BF16)

        def now():
            acc[...] += jnp.dot(o, wo_v[pl.ds(_aligned(j * _CH, _CH), _CH), :], preferred_element_type=_F32)

        def later():
            ocol[j // _DSTEP] = _columns(jnp.sum(o.astype(_F32), axis=0, keepdims=True))

        if isinstance(j, int):
            assert j >= _DSTEP * _NDEF
            now()
        else:
            deferred = jnp.logical_and(j % _DSTEP == 0, j < _DSTEP * _NDEF)
            pl.when(deferred)(later)
            pl.when(jnp.logical_not(deferred))(now)

    def k_chunk(where, c, first=False, last=False):
        for u in range(_NU):
            tick(where, c, u)
            if u % TPS == 0 and not first:
                k_step(c - 1, u // TPS)
            if u == _NU - 2 and not last:
                q_tile(c)

    def k_body(c, carry):
        k_chunk(lambda dc: (k_hbm, c + dc), c)

        @pl.when(c % CPG == 0)
        def _():
            softmax(c // CPG - 1)
        return carry

    k_chunk(where_static(0), 0, first=True)
    jax.lax.fori_loop(1, NCH - 2, k_body, 0)
    for c in range(NCH - 2, NCH + 1):
        k_chunk(where_static(c), c, last=c == NCH)
    softmax(NG - 1)

    def v_body(j, carry):
        o = None
        for u in range(_NU):
            tick(lambda dc: (v_hbm, j + dc), NCH + j, u)
            if u % TPS == 0:
                o = v_step(j - 1, u // TPS, o)
        v_finish(j - 1, o)
        return carry

    jax.lax.fori_loop(1, NCH - 2, v_body, 0)
    nleft = _AHEAD - _LAG + 1
    for j in range(NCH - 2, NCH):
        o = None
        for u in range(_NU):
            tick(where_static(NCH + j), NCH + j, u)
            k = nleft - ((NCH - j) * _NU - u) + 1
            if k > 0:
                d_issue(k * _AHEAD // nleft, k * _DEF_HI_AHEAD // nleft)
            if u % TPS == 0:
                o = v_step(j - 1, u // TPS, o)
            if j == NCH - 1 and u == TPS - 1:
                x = jnp.broadcast_to(x_v[0].astype(_F32), (8, D))
                ga = mod_v[:, 2 * D:3 * D]
                f = 1.0 + mod_v[:, 4 * D:5 * D]
                g = gsh[...]
                x1 = x + ga * _allsum8(acc[...])
                m1, sf, sg, sff, sfg, sgg = [_mean(t) for t in (x1, f, g, f * f, f * g, g * g)]
            if j == NCH - 1 and u == 2 * TPS - 1:
                r1 = jax.lax.rsqrt(_mean((x1 - m1) * (x1 - m1)) + _EPS)
                xs = (x - m1) * r1
                gs = ga * r1
                eps1 = _EPS * r1 * r1
        v_finish(j - 1, o)

    def d_work(i):
        for r0, nr, c0, nc in _rects(D, *units_d[i][0]):
            oc = ocol[r0 // _CH // _DSTEP, pl.ds(r0 % _CH, nr), :].reshape(nr // 8, 8, 128)
            for c in range(c0, c0 + nc, 128):
                w = wo_v[r0:r0 + nr, c:c + 128].astype(_F32).reshape(nr // 8, 8, 128)
                accd[c // 128] = accd[c // 128] + jnp.sum(w * oc, axis=0)

    o = None
    done = 0
    for i in range(len(units_d)):
        for p in units_d[i][1]:
            piece(p, d_sems.at[i]).wait()
        d_issue(i + 1 + _AHEAD, i + 1 + _DEF_HI_AHEAD)
        if i in (0, 4):
            for s in range(i // 4 * _STEPS // 2, (i // 4 + 1) * _STEPS // 2):
                o = v_step(NCH - 1, s, o)
        if i == 8:
            v_finish(NCH - 1, o)
        if i == 10:
            accd = [acc[:, t * 128:(t + 1) * 128] for t in range(NT)]
        if i >= 10:
            while done <= i:
                d_work(done)
                done += 1

    attn = _allsum8(jnp.concatenate(accd, axis=1))
    x1 = x + ga * attn
    a = xs + gs * attn
    e = a * f
    sa, saa, se, see, sef, seg = [_mean(t) for t in (a, a * a, e, e * e, e * f, e * g)]
    r = jax.lax.rsqrt(jnp.maximum(saa - sa * sa, 0.0) + eps1)
    m2 = r * (se - sa * sf) + sg
    ms2 = r * (r * (see - sa * (2.0 * sef - sa * sff)) + 2.0 * (seg - sa * sfg)) + sgg
    r2 = jax.lax.rsqrt(jnp.maximum(ms2 - m2 * m2, 0.0) + _EPS)
    h3 = ((e - sa * f) * r + (g - m2)) * r2

    ys = [None] * NT
    gb = [None] * NT

    def tanh_tile(i, ht):
        v = (w1b[i * 128:(i + 1) * 128, :].reshape(16, 8, 128) * ht
             + b1b[i * 128:(i + 1) * 128, :].reshape(16, 8, 128))
        return jnp.tanh(v * (v * v + k0 / alpha)).reshape(128, 128)

    def reduce_tile(i, t, th):
        part = jnp.dot(ab_v[:, i * 128:(i + 1) * 128].astype(th.dtype), th, preferred_element_type=_F32)
        ys[t] = part if ys[t] is None else part + ys[t]

    def gate_tile(t, r0):
        part = jnp.dot(sc_v[:, r0:r0 + 128].astype(_BF16),
                       wm_v[r0:r0 + 128, 5 * D + t * 128:5 * D + (t + 1) * 128], preferred_element_type=_F32)
        gb[t] = part + gb[t]

    for i in range(NB - 2):
        older = list(ys)
        for t in range(NT):
            reduce_tile(i, t, tanh_tile(i, h3[:, t * 128:(t + 1) * 128]))
    for t in range(NT):
        ht = jnp.where(older[t] > inf_v[...], 0.0, h3[:, t * 128:(t + 1) * 128])
        th_v[:, t * 128:(t + 1) * 128] = tanh_tile(NB - 2, ht)

    gb_cp.wait()
    n = D - _GB_MXU
    for t in range(NT):
        w = wm_v[_GB_MXU:D, 5 * D + t * 128:5 * D + (t + 1) * 128].astype(_F32)
        p3 = (w * scb[...]).reshape(n // 8, 8, 128)
        gb[t] = _allsum8(jnp.sum(p3[:n // 16] + p3[n // 16:], axis=0))
    pending = [functools.partial(lambda t: reduce_tile(
        NB - 2, t, th_v[:, t * 128:(t + 1) * 128].astype(_BF16)), t) for t in range(NT)]
    pending += [functools.partial(gate_tile, t, r0) for r0 in range(0, _GB_MXU, 128) for t in range(NT)]
    per = -(-len(pending) // NT)
    for t in range(NT):
        for fn in pending[t * per:(t + 1) * per]:
            fn()
        reduce_tile(NB - 1, t, tanh_tile(NB - 1, h3[:, t * 128:(t + 1) * 128]))

    lin = lin_v[...]
    outs = []
    for t in range(NT):
        yy = ys[t] + lin
        y = h3[0:1, t * 128:(t + 1) * 128] * (yy[0:1] + yy[1:2]) + (yy[2:3] + yy[3:4])
        outs.append(x1[0:1, t * 128:(t + 1) * 128] + gb[t][0:1] * y)
    o_ref[0] = jnp.concatenate(outs, axis=1).astype(o_ref.dtype)


@jax.jit
def pallas_adaLN_cond__sliding_block_cached__mixer_token_mlp__decode_kernel(
    A_x: jax.Array,
    A_k_cache: jax.Array,
    A_v_cache: jax.Array,
    A_wq: jax.Array,
    A_wo: jax.Array,
    B_x: jax.Array,
    B_w1: jax.Array,
    B_b1: jax.Array,
    B_w2: jax.Array,
    B_b2: jax.Array,
    c: jax.Array,
    w_mod: jax.Array,
):
    B, Sq, D = A_x.shape
    _, H, Sk, Dh = A_k_cache.shape
    F = B_w1.shape[1]
    assert B == 1 and Sq == 1 and B_w1.shape[0] == 1
    W = min(4096, max(256, Sk // 4))
    HD = H * Dh
    assert A_wq.shape == (D, HD) and W == 4096

    kt = jnp.swapaxes(A_k_cache, 2, 3).reshape(HD, Sk)
    vt = jnp.swapaxes(A_v_cache, 2, 3).reshape(HD, Sk)
    b1 = B_b1.reshape(F // 128, 128)
    w2 = B_w2.reshape(1, F)
    b2 = B_b2.reshape(1, 1)

    NG = H // _GROUP
    scratch = [
        pltpu.VMEM((1, 1, D), _BF16),
        pltpu.VMEM((1, D), _BF16),
        pltpu.VMEM((1, F), _BF16),
        pltpu.VMEM((F // 128, 128), _BF16),
        pltpu.VMEM((1, F), _BF16),
        pltpu.VMEM((1, 1), _BF16),
        pltpu.VMEM((D, 6 * D), _BF16),
        pltpu.VMEM((D, HD), _BF16),
        pltpu.VMEM((HD, D), _BF16),
        pltpu.VMEM((_RING, _CH, W), _BF16),
        pltpu.VMEM((2, _GROUP, _CH), _F32),
        pltpu.VMEM((NG, _GROUP, W), _F32),
        pltpu.VMEM((NG, _GROUP, W), _F32),
        pltpu.VMEM((NG, _GROUP, 128), _F32),
        pltpu.VMEM((_GROUP, D), _F32),
        pltpu.VMEM((8, 5 * D), _F32),
        pltpu.VMEM((8, D), _F32),
        pltpu.VMEM((8, D), _F32),
        pltpu.VMEM((F, 128), _F32),
        pltpu.VMEM((F, 128), _F32),
        pltpu.VMEM((8, F), _F32),
        pltpu.VMEM((8, 128), _F32),
        pltpu.VMEM((D - _GB_MXU, 128), _F32),
        pltpu.VMEM((_NDEF, _CH, 128), _F32),
        pltpu.VMEM((8, D), _F32),
        pltpu.VMEM((128, D), _F32),
        pltpu.VMEM((8, 128), _F32),
        pltpu.SemaphoreType.DMA((6,)),
        pltpu.SemaphoreType.DMA((_AHEAD,)),
        pltpu.SemaphoreType.DMA((2 * _NU,)),
        pltpu.SemaphoreType.DMA((1,)),
        pltpu.SemaphoreType.DMA((3 * _NDEF,)),
    ]
    return pl.pallas_call(
        functools.partial(_kernel, D=D, H=H, Dh=Dh, Sk=Sk, W=W, F=F),
        out_shape=jax.ShapeDtypeStruct(A_x.shape, A_x.dtype),
        in_specs=[pl.BlockSpec(memory_space=pl.ANY)] * 11,
        out_specs=pl.BlockSpec(memory_space=pltpu.VMEM),
        scratch_shapes=scratch,
        compiler_params=pltpu.CompilerParams(
            vmem_limit_bytes=64 * 1024 * 1024,
            disable_bounds_checks=True,
            disable_semaphore_checks=True),
    )(A_x, kt, vt, A_wq, A_wo, B_w1, b1, w2, b2, c, w_mod)
```

```python
import functools
import math

import jax
import jax.numpy as jnp
import jax.experimental.pallas as pl
import jax.experimental.pallas.tpu as pltpu

_F32 = jnp.float32
_BF16 = jnp.bfloat16

_EPS = 1e-05
_GROUP = 8
_CH = 128
_RING = 4
_UR = 8
_NU = _CH // _UR
_AHEAD = 21
_LAG = 5
_PA, _PP = 1792, 384
_STEPS = 4
_WIN = 32
_WIN_HI = 3
_OFF_W, _OFF_M = 17, 28
_NDEF, _DSTEP = 8, 4
_DEF_HI_AHEAD = 16
_GB_MXU = 384
_PARK, _LATE = 5, 4


def _rects(ncols, t0, t1):
    tpr = ncols // 128
    out = []
    while t0 < t1:
        g, c = divmod(t0, tpr)
        if c == 0 and t1 - t0 >= tpr:
            n = (t1 - t0) // tpr
            out.append((g * 8, n * 8, 0, ncols))
            t0 += n * tpr
        else:
            e = min(tpr, c + (t1 - t0))
            out.append((g * 8, 8, c * 128, (e - c) * 128))
            t0 += e - c
    return out


def _unit(src, dst, ncols, cmax, spans):
    tiles = [t for a, b in spans for t in range(a, b) if (t % (ncols // 128)) * 128 < cmax]
    n_hi = _WIN_HI if len(tiles) > 2 * _WIN_HI else 0
    pieces = []
    for part, prio in ((tiles[:len(tiles) - n_hi], 1), (tiles[len(tiles) - n_hi:], 0)):
        i = 0
        while i < len(part):
            k = i
            while k + 1 < len(part) and part[k + 1] == part[k] + 1:
                k += 1
            pieces += [(src, dst) + r + (prio,) for r in _rects(ncols, part[i], part[k] + 1)]
            i = k + 1
    return pieces


def _windows(src, dst, shape, off, cmax, skip=()):
    nt = shape[0] // 8 * (shape[1] // 128)
    starts = list(range(off - _WIN, nt, _WIN))
    out = []
    for b in range(8):
        for s in starts[b::8]:
            spans = [(max(s, 0), min(s + _WIN, nt))]
            for h0, h1 in skip:
                spans = [x for p, q in spans for x in ((p, min(q, h0)), (max(p, h1), q)) if x[0] < x[1]]
            u = _unit(src, dst, shape[1], cmax, spans)
            if u:
                out.append(u)
    return out


def _interleave(*lists):
    items = sorted(((k + 0.5) / len(p), n, k) for n, p in enumerate(lists) for k in range(len(p)))
    return [lists[n][k] for _, n, k in items]


def _mean(v):
    return jnp.sum(v, axis=-1, keepdims=True) * (1.0 / v.shape[-1])


def _layernorm(v):
    d = v - _mean(v)
    return d * jax.lax.rsqrt(_mean(d * d) + _EPS)


def _allsum8(v):
    v = v + pltpu.roll(v, 4, 0)
    v = v + pltpu.roll(v, 2, 0)
    return v + pltpu.roll(v, 1, 0)


def _columns(row):
    return jnp.broadcast_to(row, (128, 128)).T


def _aligned(i, n):
    return i if isinstance(i, int) else pl.multiple_of(i, n)


def _kernel(
    x_hbm, k_hbm, v_hbm, wq_hbm, wo_hbm, w1_hbm, b1_hbm, w2_hbm, b2_hbm, c_hbm, wm_hbm,
    o_ref,
    x_v, c_v, w1_v, b1_v, w2_v, b2_v, wm_v, wq_v, wo_v, ring, qbd, s_acc, p_buf, linv, acc,
    mod_v, h_v, sc_v, w1b, b1b, ab_v, lin_v, scb, ocol, gsh, th_v, inf_v,
    small_sems, w_sems, kv_sems, g_sem, d_sems,
    *, D, H, Dh, Sk, W, F,
):
    HD = H * Dh
    NG = H // _GROUP
    NCH = HD // _CH
    CPG = _GROUP * Dh // _CH
    CW = W // _STEPS
    TPS = _NU // _STEPS
    NT = D // 128
    NB = F // 128
    scale = Dh ** (-0.5)
    k0 = math.sqrt(2.0 / math.pi)
    alpha = (k0 * 0.044715) ** (1.0 / 3.0)

    def kv_piece(src, j, c, u, c0, nc):
        r = _aligned(j * _CH + u * _UR, _UR)
        return pltpu.make_async_copy(
            src.at[pl.ds(r, _UR), pl.ds(Sk - W + c0, nc)],
            ring.at[c % _RING, pl.ds(u * _UR, _UR), pl.ds(c0, nc)],
            kv_sems.at[(c % 2) * _NU + u])

    def kv_issue(where, c, u):
        dc, uu = divmod(u, _NU)
        t = where(dc)
        if t is not None:
            kv_piece(t[0], t[1], c + dc, uu, 0, _PA).start(priority=1)
            kv_piece(t[0], t[1], c + dc, uu, _PA, _PP).start(priority=0)
        dc, uu = divmod(u - _LAG, _NU)
        t = where(dc) if dc >= 0 else None
        if t is not None:
            kv_piece(t[0], t[1], c + dc, uu, _PA + _PP, W - _PA - _PP).start(priority=1)

    def where_static(c):
        def where(dc):
            if c + dc < NCH:
                return (k_hbm, c + dc)
            if c + dc < 2 * NCH:
                return (v_hbm, c + dc - NCH)
            return None
        return where

    def tick(where, c, u):
        kv_piece(k_hbm, 0, c, u, 0, W).wait()
        kv_issue(where, c, u + _AHEAD)

    tpc = _CH // 8 * NT
    holes = [(j * _DSTEP * tpc, (j * _DSTEP + 1) * tpc) for j in range(_NDEF)]
    units_mq = _interleave(_windows(wm_hbm, wm_v, (D, 6 * D), _OFF_M, 5 * D),
                           _windows(wq_hbm, wq_v, (D, HD), _OFF_W, HD))
    pre = units_mq + _windows(wo_hbm, wo_v, (HD, D), _OFF_W, D, holes)
    units_d = []
    for p in (1, 2, 0):
        for h0, h1 in holes:
            cuts = [h0] + [t for t in range(h0 + 1, h1) if t % _WIN == _OFF_W] + [h1]
            assert len(cuts) == 4
            span = (cuts[p], cuts[p + 1])
            units_d.append((span, _unit(wo_hbm, wo_v, D, D, [span])))

    def piece(p, sem):
        src, dst, r0, nr, c0, nc, _ = p
        return pltpu.make_async_copy(
            src.at[pl.ds(r0, nr), pl.ds(c0, nc)], dst.at[pl.ds(r0, nr), pl.ds(c0, nc)], sem)

    def w_start(i):
        for p in pre[i]:
            piece(p, w_sems.at[i % _AHEAD]).start(priority=p[-1])

    def w_wait(i):
        for p in pre[i]:
            piece(p, w_sems.at[i % _AHEAD]).wait()

    small = [(c_hbm, c_v), (x_hbm, x_v), (w1_hbm, w1_v), (b1_hbm, b1_v), (w2_hbm, w2_v), (b2_hbm, b2_v)]
    small_cp = [pltpu.make_async_copy(s, d, small_sems.at[i]) for i, (s, d) in enumerate(small)]
    gb_cp = pltpu.make_async_copy(
        wm_hbm.at[:, pl.ds(5 * D, D)], wm_v.at[:, pl.ds(5 * D, D)], g_sem.at[0])
    d_next = [0, 0]

    def d_issue(upto_lo, upto_hi):
        while d_next[0] < upto_lo:
            i = d_next[0]
            if i < len(units_d):
                for p in units_d[i][1]:
                    if p[-1] == 1:
                        piece(p, d_sems.at[i]).start(priority=1)
            elif i == len(units_d):
                gb_cp.start(priority=1)
            d_next[0] += 1
        while d_next[1] < min(upto_hi, len(units_d)):
            i = d_next[1]
            for p in units_d[i][1]:
                if p[-1] == 0:
                    piece(p, d_sems.at[i]).start(priority=0)
            d_next[1] += 1

    def prep_small():
        c = c_v[...].astype(_F32)
        sc = (c * jax.nn.sigmoid(c)).astype(_BF16).astype(_F32)
        sc_v[...] = jnp.broadcast_to(sc, (8, D))
        s_acc[...] = jnp.zeros(s_acc.shape, _F32)
        acc[...] = jnp.zeros(acc.shape, _F32)
        inf_v[...] = jnp.full(inf_v.shape, jnp.inf, _F32)

    def prep_scb(r):
        scb[r - _GB_MXU:r - _GB_MXU + 128, :] = _columns(sc_v[0:1, r:r + 128])

    def prep_mlp(i):
        w1 = w1_v[:, i * 128:(i + 1) * 128].astype(_F32)
        w2 = w2_v[:, i * 128:(i + 1) * 128].astype(_F32)
        b1 = b1_v[...].astype(_F32)[i:i + 1, :]
        w1b[i * 128:(i + 1) * 128, :] = _columns(w1 * alpha)
        b1b[i * 128:(i + 1) * 128, :] = _columns(b1 * alpha)
        a = 0.5 * w2 * w1
        b = 0.5 * w2 * b1
        a_hi = a.astype(_BF16).astype(_F32)
        b_hi = b.astype(_BF16).astype(_F32)
        sub = jax.lax.broadcasted_iota(jnp.int32, (8, 128), 0)
        ab_v[:, i * 128:(i + 1) * 128] = jnp.where(
            sub == 0, a_hi, jnp.where(sub == 1, a - a_hi, jnp.where(
                sub == 2, b_hi, jnp.where(sub == 3, b - b_hi, 0.0))))

    def prep_lin():
        sub = jax.lax.broadcasted_iota(jnp.int32, (8, 128), 0)
        tot = jnp.broadcast_to(jnp.sum(ab_v[...], axis=1, keepdims=True), (8, 128))
        lin_v[...] = tot + jnp.where(sub == 2, jnp.broadcast_to(b2_v[...].astype(_F32), (8, 128)), 0.0)

    def mod_tiles(t0, t1):
        mod_v[:, t0 * 128:t1 * 128] = jnp.dot(
            sc_v[...].astype(_BF16), wm_v[:, t0 * 128:t1 * 128], preferred_element_type=_F32)

    def make_h():
        x = jnp.broadcast_to(x_v[0].astype(_F32), (8, D))
        h_v[...] = _layernorm(x) * (1.0 + mod_v[:, D:2 * D]) + mod_v[:, 0:D]
        sb = mod_v[:, 3 * D:4 * D]
        gsh[...] = sb - _mean(sb)

    work = {}
    items = [prep_small] + [functools.partial(prep_scb, r) for r in range(_GB_MXU, D, 128)]
    items += [functools.partial(prep_mlp, i) for i in range(NB)] + [prep_lin]
    for k, fn in enumerate(items):
        work[12 + 6 * k] = fn
    assert 12 + 6 * len(items) <= len(units_mq)
    items = [functools.partial(mod_tiles, t, min(t + 2, 5 * NT)) for t in range(0, 5 * NT, 2)] + [make_h]
    for k, fn in enumerate(items):
        work[len(units_mq) + 5 * k] = fn
    assert len(units_mq) + 5 * len(items) <= len(pre)

    for i in range(_AHEAD):
        w_start(i)
    for cp in small_cp:
        cp.start()
    for i in range(len(pre)):
        w_wait(i)
        if i + _AHEAD < len(pre):
            w_start(i + _AHEAD)
        else:
            kv_issue(where_static(0), 0, i + _AHEAD - len(pre))
        if i == 8:
            for cp in small_cp:
                cp.wait()
        if i in work:
            work[i]()

    def diag_mask(j):
        lo = jax.lax.broadcasted_iota(jnp.int32, (_GROUP, _CH), 0) * Dh - (j % CPG) * _CH
        col = jax.lax.broadcasted_iota(jnp.int32, (_GROUP, _CH), 1)
        return (col >= lo) & (col < lo + Dh)

    def q_tile(j):
        q = jnp.dot(h_v[...].astype(_BF16), wq_v[:, pl.ds(_aligned(j * _CH, _CH), _CH)],
                    preferred_element_type=_F32)
        qbd[j % 2] = jnp.where(diag_mask(j), q, 0.0)

    def k_step(j, s):
        cols = pl.ds(s * CW, CW)
        s_acc[j // CPG, :, cols] += jnp.dot(
            qbd[j % 2].astype(_BF16), ring[j % _RING, :, cols], preferred_element_type=_F32)

    def softmax(g):
        s = s_acc[g]
        m = jnp.max(s, axis=-1, keepdims=True)
        p = jnp.exp((s - m) * scale)
        p_buf[g] = p
        linv[g] = jnp.broadcast_to(1.0 / jnp.sum(p, axis=-1, keepdims=True), (_GROUP, 128))

    def v_step(j, s, o):
        cols = pl.ds(s * CW, CW)
        part = jax.lax.dot_general(
            p_buf[j // CPG, :, cols].astype(_BF16), ring[(j + NCH) % _RING, :, cols],
            (((1,), (1,)), ((), ())), preferred_element_type=_F32)
        return part if o is None else part + o

    def v_finish(j, o):
        o = jnp.where(diag_mask(j), o * linv[j // CPG], 0.0).astype(_BF16)

        def now():
            acc[...] += jnp.dot(o, wo_v[pl.ds(_aligned(j * _CH, _CH), _CH), :], preferred_element_type=_F32)

        def later():
            ocol[j // _DSTEP] = _columns(jnp.sum(o.astype(_F32), axis=0, keepdims=True))

        if isinstance(j, int):
            assert j >= _DSTEP * _NDEF
            now()
        else:
            deferred = jnp.logical_and(j % _DSTEP == 0, j < _DSTEP * _NDEF)
            pl.when(deferred)(later)
            pl.when(jnp.logical_not(deferred))(now)

    def k_chunk(where, c, first=False, last=False):
        for u in range(_NU):
            tick(where, c, u)
            if u % TPS == 0 and not first:
                k_step(c - 1, u // TPS)
            if u == _NU - 2 and not last:
                q_tile(c)

    def k_body(c, carry):
        k_chunk(lambda dc: (k_hbm, c + dc), c)

        @pl.when(c % CPG == 0)
        def _():
            softmax(c // CPG - 1)
        return carry

    k_chunk(where_static(0), 0, first=True)
    jax.lax.fori_loop(1, NCH - 2, k_body, 0)
    for c in range(NCH - 2, NCH + 1):
        k_chunk(where_static(c), c, last=c == NCH)
    softmax(NG - 1)

    def v_body(j, carry):
        o = None
        for u in range(_NU):
            tick(lambda dc: (v_hbm, j + dc), NCH + j, u)
            if u % TPS == 0:
                o = v_step(j - 1, u // TPS, o)
        v_finish(j - 1, o)
        return carry

    jax.lax.fori_loop(1, NCH - 2, v_body, 0)
    nleft = _AHEAD - _LAG + 1
    for j in range(NCH - 2, NCH):
        o = None
        for u in range(_NU):
            tick(where_static(NCH + j), NCH + j, u)
            k = nleft - ((NCH - j) * _NU - u) + 1
            if k > 0:
                d_issue(k * _AHEAD // nleft, k * _DEF_HI_AHEAD // nleft)
            if u % TPS == 0:
                o = v_step(j - 1, u // TPS, o)
            if j == NCH - 1 and u == TPS - 1:
                x = jnp.broadcast_to(x_v[0].astype(_F32), (8, D))
                ga = mod_v[:, 2 * D:3 * D]
                f = 1.0 + mod_v[:, 4 * D:5 * D]
                g = gsh[...]
                x1 = x + ga * _allsum8(acc[...])
                m1, sf, sg, sff, sfg, sgg = [_mean(t) for t in (x1, f, g, f * f, f * g, g * g)]
            if j == NCH - 1 and u == 2 * TPS - 1:
                r1 = jax.lax.rsqrt(_mean((x1 - m1) * (x1 - m1)) + _EPS)
                xs = (x - m1) * r1
                gs = ga * r1
                eps1 = _EPS * r1 * r1
        v_finish(j - 1, o)

    def d_work(i):
        for r0, nr, c0, nc in _rects(D, *units_d[i][0]):
            oc = ocol[r0 // _CH // _DSTEP, pl.ds(r0 % _CH, nr), :].reshape(nr // 8, 8, 128)
            for c in range(c0, c0 + nc, 128):
                w = wo_v[r0:r0 + nr, c:c + 128].astype(_F32).reshape(nr // 8, 8, 128)
                accd[c // 128] = accd[c // 128] + jnp.sum(w * oc, axis=0)

    o = None
    done = 0
    for i in range(len(units_d)):
        for p in units_d[i][1]:
            piece(p, d_sems.at[i]).wait()
        d_issue(i + 1 + _AHEAD, i + 1 + _DEF_HI_AHEAD)
        if i in (0, 4):
            for s in range(i // 4 * _STEPS // 2, (i // 4 + 1) * _STEPS // 2):
                o = v_step(NCH - 1, s, o)
        if i == 8:
            v_finish(NCH - 1, o)
        if i == 10:
            accd = [acc[:, t * 128:(t + 1) * 128] for t in range(NT)]
        if i >= 10:
            while done <= i:
                d_work(done)
                done += 1

    attn = _allsum8(jnp.concatenate(accd, axis=1))
    x1 = x + ga * attn
    a = xs + gs * attn
    e = a * f
    sa, saa, se, see, sef, seg = [_mean(t) for t in (a, a * a, e, e * e, e * f, e * g)]
    r = jax.lax.rsqrt(jnp.maximum(saa - sa * sa, 0.0) + eps1)
    m2 = r * (se - sa * sf) + sg
    ms2 = r * (r * (see - sa * (2.0 * sef - sa * sff)) + 2.0 * (seg - sa * sfg)) + sgg
    r2 = jax.lax.rsqrt(jnp.maximum(ms2 - m2 * m2, 0.0) + _EPS)
    h3 = ((e - sa * f) * r + (g - m2)) * r2

    ys = [None] * NT
    gb = [None] * NT

    def tanh_tile(i, ht):
        v = (w1b[i * 128:(i + 1) * 128, :].reshape(16, 8, 128) * ht
             + b1b[i * 128:(i + 1) * 128, :].reshape(16, 8, 128))
        return jnp.tanh(v * (v * v + k0 / alpha)).reshape(128, 128)

    def reduce_tile(i, t, th):
        part = jnp.dot(ab_v[:, i * 128:(i + 1) * 128].astype(th.dtype), th, preferred_element_type=_F32)
        ys[t] = part if ys[t] is None else part + ys[t]

    def gate_tile(t, r0):
        part = jnp.dot(sc_v[:, r0:r0 + 128].astype(_BF16),
                       wm_v[r0:r0 + 128, 5 * D + t * 128:5 * D + (t + 1) * 128], preferred_element_type=_F32)
        gb[t] = part + gb[t]

    tiles = [(i, t) for i in range(NB) for t in range(NT)]
    n_direct = len(tiles) - _PARK - _LATE
    parked, late = tiles[n_direct:n_direct + _PARK], tiles[n_direct + _PARK:]
    sums = []
    for i, t in tiles[:n_direct]:
        reduce_tile(i, t, tanh_tile(i, h3[:, t * 128:(t + 1) * 128]))
        sums.append(ys[t])
    for k, (i, t) in enumerate(parked):
        ht = jnp.where(sums[n_direct - 2 * _PARK + k] > inf_v[...], 0.0, h3[:, t * 128:(t + 1) * 128])
        th_v[:, k * 128:(k + 1) * 128] = tanh_tile(i, ht)

    gb_cp.wait()
    n = D - _GB_MXU
    for t in range(NT):
        w = wm_v[_GB_MXU:D, 5 * D + t * 128:5 * D + (t + 1) * 128].astype(_F32)
        p3 = (w * scb[...]).reshape(n // 8, 8, 128)
        gb[t] = _allsum8(jnp.sum(p3[:n // 16] + p3[n // 16:], axis=0))

    def unpark(k, i, t):
        reduce_tile(i, t, th_v[:, k * 128:(k + 1) * 128].astype(_BF16))

    pending = [functools.partial(unpark, k, i, t) for k, (i, t) in enumerate(parked)]
    pending += [functools.partial(gate_tile, t, r0) for r0 in range(0, _GB_MXU, 128) for t in range(NT)]
    per = -(-len(pending) // len(late))
    for k, (i, t) in enumerate(late):
        for fn in pending[k * per:(k + 1) * per]:
            fn()
        reduce_tile(i, t, tanh_tile(i, h3[:, t * 128:(t + 1) * 128]))

    lin = lin_v[...]
    outs = []
    for t in range(NT):
        yy = ys[t] + lin
        y = h3[0:1, t * 128:(t + 1) * 128] * (yy[0:1] + yy[1:2]) + (yy[2:3] + yy[3:4])
        outs.append(x1[0:1, t * 128:(t + 1) * 128] + gb[t][0:1] * y)
    o_ref[0] = jnp.concatenate(outs, axis=1).astype(o_ref.dtype)


@jax.jit
def pallas_adaLN_cond__sliding_block_cached__mixer_token_mlp__decode_kernel(
    A_x: jax.Array,
    A_k_cache: jax.Array,
    A_v_cache: jax.Array,
    A_wq: jax.Array,
    A_wo: jax.Array,
    B_x: jax.Array,
    B_w1: jax.Array,
    B_b1: jax.Array,
    B_w2: jax.Array,
    B_b2: jax.Array,
    c: jax.Array,
    w_mod: jax.Array,
):
    B, Sq, D = A_x.shape
    _, H, Sk, Dh = A_k_cache.shape
    F = B_w1.shape[1]
    assert B == 1 and Sq == 1 and B_w1.shape[0] == 1
    W = min(4096, max(256, Sk // 4))
    HD = H * Dh
    assert A_wq.shape == (D, HD) and W == 4096

    kt = jnp.swapaxes(A_k_cache, 2, 3).reshape(HD, Sk)
    vt = jnp.swapaxes(A_v_cache, 2, 3).reshape(HD, Sk)
    b1 = B_b1.reshape(F // 128, 128)
    w2 = B_w2.reshape(1, F)
    b2 = B_b2.reshape(1, 1)

    NG = H // _GROUP
    scratch = [
        pltpu.VMEM((1, 1, D), _BF16),
        pltpu.VMEM((1, D), _BF16),
        pltpu.VMEM((1, F), _BF16),
        pltpu.VMEM((F // 128, 128), _BF16),
        pltpu.VMEM((1, F), _BF16),
        pltpu.VMEM((1, 1), _BF16),
        pltpu.VMEM((D, 6 * D), _BF16),
        pltpu.VMEM((D, HD), _BF16),
        pltpu.VMEM((HD, D), _BF16),
        pltpu.VMEM((_RING, _CH, W), _BF16),
        pltpu.VMEM((2, _GROUP, _CH), _F32),
        pltpu.VMEM((NG, _GROUP, W), _F32),
        pltpu.VMEM((NG, _GROUP, W), _F32),
        pltpu.VMEM((NG, _GROUP, 128), _F32),
        pltpu.VMEM((_GROUP, D), _F32),
        pltpu.VMEM((8, 5 * D), _F32),
        pltpu.VMEM((8, D), _F32),
        pltpu.VMEM((8, D), _F32),
        pltpu.VMEM((F, 128), _F32),
        pltpu.VMEM((F, 128), _F32),
        pltpu.VMEM((8, F), _F32),
        pltpu.VMEM((8, 128), _F32),
        pltpu.VMEM((D - _GB_MXU, 128), _F32),
        pltpu.VMEM((_NDEF, _CH, 128), _F32),
        pltpu.VMEM((8, D), _F32),
        pltpu.VMEM((128, 128 * _PARK), _F32),
        pltpu.VMEM((8, 128), _F32),
        pltpu.SemaphoreType.DMA((6,)),
        pltpu.SemaphoreType.DMA((_AHEAD,)),
        pltpu.SemaphoreType.DMA((2 * _NU,)),
        pltpu.SemaphoreType.DMA((1,)),
        pltpu.SemaphoreType.DMA((3 * _NDEF,)),
    ]
    return pl.pallas_call(
        functools.partial(_kernel, D=D, H=H, Dh=Dh, Sk=Sk, W=W, F=F),
        out_shape=jax.ShapeDtypeStruct(A_x.shape, A_x.dtype),
        in_specs=[pl.BlockSpec(memory_space=pl.ANY)] * 11,
        out_specs=pl.BlockSpec(memory_space=pltpu.VMEM),
        scratch_shapes=scratch,
        compiler_params=pltpu.CompilerParams(
            vmem_limit_bytes=64 * 1024 * 1024,
            disable_bounds_checks=True,
            disable_semaphore_checks=True),
    )(A_x, kt, vt, A_wq, A_wo, B_w1, b1, w2, b2, c, w_mod)
```

```python
import functools
import math

import jax
import jax.numpy as jnp
import jax.experimental.pallas as pl
import jax.experimental.pallas.tpu as pltpu

_F32 = jnp.float32
_BF16 = jnp.bfloat16

_EPS = 1e-05
_GROUP = 8
_CH = 128
_RING = 4
_UR = 8
_NU = _CH // _UR
_AHEAD = 21
_LAG = 5
_PA, _PP = 1792, 384
_STEPS = 4
_WIN = 32
_WIN_HI = 3
_OFF_W, _OFF_M = 17, 28
_NDEF, _DSTEP = 8, 4
_DEF_HI_AHEAD = 16
_GB_MXU = 384
_COND = 4096.0
_PARK, _LATE = 5, 4


def _rects(ncols, t0, t1):
    tpr = ncols // 128
    out = []
    while t0 < t1:
        g, c = divmod(t0, tpr)
        if c == 0 and t1 - t0 >= tpr:
            n = (t1 - t0) // tpr
            out.append((g * 8, n * 8, 0, ncols))
            t0 += n * tpr
        else:
            e = min(tpr, c + (t1 - t0))
            out.append((g * 8, 8, c * 128, (e - c) * 128))
            t0 += e - c
    return out


def _unit(src, dst, ncols, cmax, spans):
    tiles = [t for a, b in spans for t in range(a, b) if (t % (ncols // 128)) * 128 < cmax]
    n_hi = _WIN_HI if len(tiles) > 2 * _WIN_HI else 0
    pieces = []
    for part, prio in ((tiles[:len(tiles) - n_hi], 1), (tiles[len(tiles) - n_hi:], 0)):
        i = 0
        while i < len(part):
            k = i
            while k + 1 < len(part) and part[k + 1] == part[k] + 1:
                k += 1
            pieces += [(src, dst) + r + (prio,) for r in _rects(ncols, part[i], part[k] + 1)]
            i = k + 1
    return pieces


def _windows(src, dst, shape, off, cmax, skip=()):
    nt = shape[0] // 8 * (shape[1] // 128)
    starts = list(range(off - _WIN, nt, _WIN))
    out = []
    for b in range(8):
        for s in starts[b::8]:
            spans = [(max(s, 0), min(s + _WIN, nt))]
            for h0, h1 in skip:
                spans = [x for p, q in spans for x in ((p, min(q, h0)), (max(p, h1), q)) if x[0] < x[1]]
            u = _unit(src, dst, shape[1], cmax, spans)
            if u:
                out.append(u)
    return out


def _interleave(*lists):
    items = sorted(((k + 0.5) / len(p), n, k) for n, p in enumerate(lists) for k in range(len(p)))
    return [lists[n][k] for _, n, k in items]


def _mean(v):
    return jnp.sum(v, axis=-1, keepdims=True) * (1.0 / v.shape[-1])


def _layernorm(v):
    d = v - _mean(v)
    return d * jax.lax.rsqrt(_mean(d * d) + _EPS)


def _allsum8(v):
    v = v + pltpu.roll(v, 4, 0)
    v = v + pltpu.roll(v, 2, 0)
    return v + pltpu.roll(v, 1, 0)


def _columns(row):
    return jnp.broadcast_to(row, (128, 128)).T


def _aligned(i, n):
    return i if isinstance(i, int) else pl.multiple_of(i, n)


def _kernel(
    x_hbm, k_hbm, v_hbm, wq_hbm, wo_hbm, w1_hbm, b1_hbm, w2_hbm, b2_hbm, c_hbm, wm_hbm,
    o_ref,
    x_v, c_v, w1_v, b1_v, w2_v, b2_v, wm_v, wq_v, wo_v, ring, qbd, s_acc, p_buf, linv, acc,
    mod_v, h_v, sc_v, w1b, b1b, ab_v, lin_v, scb, ocol, gsh, th_v, inf_v,
    small_sems, w_sems, kv_sems, g_sem, d_sems,
    *, D, H, Dh, Sk, W, F,
):
    HD = H * Dh
    NG = H // _GROUP
    NCH = HD // _CH
    CPG = _GROUP * Dh // _CH
    CW = W // _STEPS
    TPS = _NU // _STEPS
    NT = D // 128
    NB = F // 128
    scale = Dh ** (-0.5)
    k0 = math.sqrt(2.0 / math.pi)
    alpha = (k0 * 0.044715) ** (1.0 / 3.0)

    def kv_piece(src, j, c, u, c0, nc):
        r = _aligned(j * _CH + u * _UR, _UR)
        return pltpu.make_async_copy(
            src.at[pl.ds(r, _UR), pl.ds(Sk - W + c0, nc)],
            ring.at[c % _RING, pl.ds(u * _UR, _UR), pl.ds(c0, nc)],
            kv_sems.at[(c % 2) * _NU + u])

    def kv_issue(where, c, u):
        dc, uu = divmod(u, _NU)
        t = where(dc)
        if t is not None:
            kv_piece(t[0], t[1], c + dc, uu, 0, _PA).start(priority=1)
            kv_piece(t[0], t[1], c + dc, uu, _PA, _PP).start(priority=0)
        dc, uu = divmod(u - _LAG, _NU)
        t = where(dc) if dc >= 0 else None
        if t is not None:
            kv_piece(t[0], t[1], c + dc, uu, _PA + _PP, W - _PA - _PP).start(priority=1)

    def where_static(c):
        def where(dc):
            if c + dc < NCH:
                return (k_hbm, c + dc)
            if c + dc < 2 * NCH:
                return (v_hbm, c + dc - NCH)
            return None
        return where

    def tick(where, c, u):
        kv_piece(k_hbm, 0, c, u, 0, W).wait()
        kv_issue(where, c, u + _AHEAD)

    tpc = _CH // 8 * NT
    holes = [(j * _DSTEP * tpc, (j * _DSTEP + 1) * tpc) for j in range(_NDEF)]
    units_mq = _interleave(_windows(wm_hbm, wm_v, (D, 6 * D), _OFF_M, 5 * D),
                           _windows(wq_hbm, wq_v, (D, HD), _OFF_W, HD))
    pre = units_mq + _windows(wo_hbm, wo_v, (HD, D), _OFF_W, D, holes)
    units_d = []
    for p in (1, 2, 0):
        for h0, h1 in holes:
            cuts = [h0] + [t for t in range(h0 + 1, h1) if t % _WIN == _OFF_W] + [h1]
            assert len(cuts) == 4
            span = (cuts[p], cuts[p + 1])
            units_d.append((span, _unit(wo_hbm, wo_v, D, D, [span])))

    def piece(p, sem):
        src, dst, r0, nr, c0, nc, _ = p
        return pltpu.make_async_copy(
            src.at[pl.ds(r0, nr), pl.ds(c0, nc)], dst.at[pl.ds(r0, nr), pl.ds(c0, nc)], sem)

    def w_start(i):
        for p in pre[i]:
            piece(p, w_sems.at[i % _AHEAD]).start(priority=p[-1])

    def w_wait(i):
        for p in pre[i]:
            piece(p, w_sems.at[i % _AHEAD]).wait()

    small = [(c_hbm, c_v), (x_hbm, x_v), (w1_hbm, w1_v), (b1_hbm, b1_v), (w2_hbm, w2_v), (b2_hbm, b2_v)]
    small_cp = [pltpu.make_async_copy(s, d, small_sems.at[i]) for i, (s, d) in enumerate(small)]
    gb_cp = pltpu.make_async_copy(
        wm_hbm.at[:, pl.ds(5 * D, D)], wm_v.at[:, pl.ds(5 * D, D)], g_sem.at[0])
    d_next = [0, 0]

    def d_issue(upto_lo, upto_hi):
        while d_next[0] < upto_lo:
            i = d_next[0]
            if i < len(units_d):
                for p in units_d[i][1]:
                    if p[-1] == 1:
                        piece(p, d_sems.at[i]).start(priority=1)
            elif i == len(units_d):
                gb_cp.start(priority=1)
            d_next[0] += 1
        while d_next[1] < min(upto_hi, len(units_d)):
            i = d_next[1]
            for p in units_d[i][1]:
                if p[-1] == 0:
                    piece(p, d_sems.at[i]).start(priority=0)
            d_next[1] += 1

    def prep_small():
        c = c_v[...].astype(_F32)
        sc = (c * jax.nn.sigmoid(c)).astype(_BF16).astype(_F32)
        sc_v[...] = jnp.broadcast_to(sc, (8, D))
        s_acc[...] = jnp.zeros(s_acc.shape, _F32)
        acc[...] = jnp.zeros(acc.shape, _F32)
        inf_v[...] = jnp.full(inf_v.shape, jnp.inf, _F32)

    def prep_scb(r):
        scb[r - _GB_MXU:r - _GB_MXU + 128, :] = _columns(sc_v[0:1, r:r + 128])

    def prep_mlp(i):
        w1 = w1_v[:, i * 128:(i + 1) * 128].astype(_F32)
        w2 = w2_v[:, i * 128:(i + 1) * 128].astype(_F32)
        b1 = b1_v[...].astype(_F32)[i:i + 1, :]
        w1b[i * 128:(i + 1) * 128, :] = _columns(w1 * alpha)
        b1b[i * 128:(i + 1) * 128, :] = _columns(b1 * alpha)
        a = 0.5 * w2 * w1
        b = 0.5 * w2 * b1
        a_hi = a.astype(_BF16).astype(_F32)
        b_hi = b.astype(_BF16).astype(_F32)
        sub = jax.lax.broadcasted_iota(jnp.int32, (8, 128), 0)
        ab_v[:, i * 128:(i + 1) * 128] = jnp.where(
            sub == 0, a_hi, jnp.where(sub == 1, a - a_hi, jnp.where(
                sub == 2, b_hi, jnp.where(sub == 3, b - b_hi, 0.0))))

    def prep_lin():
        sub = jax.lax.broadcasted_iota(jnp.int32, (8, 128), 0)
        tot = jnp.broadcast_to(jnp.sum(ab_v[...], axis=1, keepdims=True), (8, 128))
        lin_v[...] = tot + jnp.where(sub == 2, jnp.broadcast_to(b2_v[...].astype(_F32), (8, 128)), 0.0)

    def mod_tiles(t0, t1):
        mod_v[:, t0 * 128:t1 * 128] = jnp.dot(
            sc_v[...].astype(_BF16), wm_v[:, t0 * 128:t1 * 128], preferred_element_type=_F32)

    def make_h():
        x = jnp.broadcast_to(x_v[0].astype(_F32), (8, D))
        h_v[...] = _layernorm(x) * (1.0 + mod_v[:, D:2 * D]) + mod_v[:, 0:D]
        sb = mod_v[:, 3 * D:4 * D]
        gsh[...] = sb - _mean(sb)

    work = {}
    items = [prep_small] + [functools.partial(prep_scb, r) for r in range(_GB_MXU, D, 128)]
    items += [functools.partial(prep_mlp, i) for i in range(NB)] + [prep_lin]
    for k, fn in enumerate(items):
        work[12 + 6 * k] = fn
    assert 12 + 6 * len(items) <= len(units_mq)
    items = [functools.partial(mod_tiles, t, min(t + 2, 5 * NT)) for t in range(0, 5 * NT, 2)] + [make_h]
    for k, fn in enumerate(items):
        work[len(units_mq) + 5 * k] = fn
    assert len(units_mq) + 5 * len(items) <= len(pre)

    for i in range(_AHEAD):
        w_start(i)
    for cp in small_cp:
        cp.start()
    for i in range(len(pre)):
        w_wait(i)
        if i + _AHEAD < len(pre):
            w_start(i + _AHEAD)
        else:
            kv_issue(where_static(0), 0, i + _AHEAD - len(pre))
        if i == 8:
            for cp in small_cp:
                cp.wait()
        if i in work:
            work[i]()

    def diag_mask(j):
        lo = jax.lax.broadcasted_iota(jnp.int32, (_GROUP, _CH), 0) * Dh - (j % CPG) * _CH
        col = jax.lax.broadcasted_iota(jnp.int32, (_GROUP, _CH), 1)
        return (col >= lo) & (col < lo + Dh)

    def q_tile(j):
        q = jnp.dot(h_v[...].astype(_BF16), wq_v[:, pl.ds(_aligned(j * _CH, _CH), _CH)],
                    preferred_element_type=_F32)
        qbd[j % 2] = jnp.where(diag_mask(j), q, 0.0)

    def k_step(j, s):
        cols = pl.ds(s * CW, CW)
        s_acc[j // CPG, :, cols] += jnp.dot(
            qbd[j % 2].astype(_BF16), ring[j % _RING, :, cols], preferred_element_type=_F32)

    def softmax(g):
        s = s_acc[g]
        m = jnp.max(s, axis=-1, keepdims=True)
        p = jnp.exp((s - m) * scale)
        p_buf[g] = p
        linv[g] = jnp.broadcast_to(1.0 / jnp.sum(p, axis=-1, keepdims=True), (_GROUP, 128))

    def v_step(j, s, o):
        cols = pl.ds(s * CW, CW)
        part = jax.lax.dot_general(
            p_buf[j // CPG, :, cols].astype(_BF16), ring[(j + NCH) % _RING, :, cols],
            (((1,), (1,)), ((), ())), preferred_element_type=_F32)
        return part if o is None else part + o

    def v_finish(j, o):
        o = jnp.where(diag_mask(j), o * linv[j // CPG], 0.0).astype(_BF16)

        def now():
            acc[...] += jnp.dot(o, wo_v[pl.ds(_aligned(j * _CH, _CH), _CH), :], preferred_element_type=_F32)

        def later():
            ocol[j // _DSTEP] = _columns(jnp.sum(o.astype(_F32), axis=0, keepdims=True))

        if isinstance(j, int):
            assert j >= _DSTEP * _NDEF
            now()
        else:
            deferred = jnp.logical_and(j % _DSTEP == 0, j < _DSTEP * _NDEF)
            pl.when(deferred)(later)
            pl.when(jnp.logical_not(deferred))(now)

    def k_chunk(where, c, first=False, last=False):
        for u in range(_NU):
            tick(where, c, u)
            if u % TPS == 0 and not first:
                k_step(c - 1, u // TPS)
            if u == _NU - 2 and not last:
                q_tile(c)

    def k_body(c, carry):
        k_chunk(lambda dc: (k_hbm, c + dc), c)

        @pl.when(c % CPG == 0)
        def _():
            softmax(c // CPG - 1)
        return carry

    k_chunk(where_static(0), 0, first=True)
    jax.lax.fori_loop(1, NCH - 2, k_body, 0)
    for c in range(NCH - 2, NCH + 1):
        k_chunk(where_static(c), c, last=c == NCH)
    softmax(NG - 1)

    def v_body(j, carry):
        o = None
        for u in range(_NU):
            tick(lambda dc: (v_hbm, j + dc), NCH + j, u)
            if u % TPS == 0:
                o = v_step(j - 1, u // TPS, o)
        v_finish(j - 1, o)
        return carry

    jax.lax.fori_loop(1, NCH - 2, v_body, 0)
    nleft = _AHEAD - _LAG + 1
    for j in range(NCH - 2, NCH):
        o = None
        for u in range(_NU):
            tick(where_static(NCH + j), NCH + j, u)
            k = nleft - ((NCH - j) * _NU - u) + 1
            if k > 0:
                d_issue(k * _AHEAD // nleft, k * _DEF_HI_AHEAD // nleft)
            if u % TPS == 0:
                o = v_step(j - 1, u // TPS, o)
            if j == NCH - 1 and u == TPS - 1:
                x = jnp.broadcast_to(x_v[0].astype(_F32), (8, D))
                ga = mod_v[:, 2 * D:3 * D]
                f = 1.0 + mod_v[:, 4 * D:5 * D]
                g = gsh[...]
                x1 = x + ga * _allsum8(acc[...])
                m1, sf, sg, sff, sfg, sgg = [_mean(t) for t in (x1, f, g, f * f, f * g, g * g)]
            if j == NCH - 1 and u == 2 * TPS - 1:
                r1 = jax.lax.rsqrt(_mean((x1 - m1) * (x1 - m1)) + _EPS)
                xs = (x - m1) * r1
                gs = ga * r1
                eps1 = _EPS * r1 * r1
        v_finish(j - 1, o)

    arrived = set()

    def d_work(i):
        t0, t1 = units_d[i][0]
        arrived.update(range(t0, t1))
        groups = [q for q in range(t0 // NT, (t1 - 1) // NT + 1)
                  if all(q * NT + t in arrived for t in range(NT))]
        r0, nr = groups[0] * 8, len(groups) * 8
        oc = ocol[r0 // _CH // _DSTEP, pl.ds(r0 % _CH, nr), :].reshape(nr // 8, 8, 128)
        for t in range(NT):
            w = wo_v[r0:r0 + nr, t * 128:(t + 1) * 128].astype(_F32).reshape(nr // 8, 8, 128)
            accd[t] = accd[t] + jnp.sum(w * oc, axis=0)

    o = None
    done = 0
    for i in range(len(units_d)):
        for p in units_d[i][1]:
            piece(p, d_sems.at[i]).wait()
        d_issue(i + 1 + _AHEAD, i + 1 + _DEF_HI_AHEAD)
        if i in (0, 4):
            for s in range(i // 4 * _STEPS // 2, (i // 4 + 1) * _STEPS // 2):
                o = v_step(NCH - 1, s, o)
        if i == 8:
            v_finish(NCH - 1, o)
        if i == 10:
            accd = [acc[:, t * 128:(t + 1) * 128] for t in range(NT)]
        if i >= 10:
            while done <= i:
                d_work(done)
                done += 1

    attn = _allsum8(jnp.concatenate(accd, axis=1))
    x1 = x + ga * attn
    a = xs + gs * attn
    e = a * f
    sa, saa, se, see, sef, seg = [_mean(t) for t in (a, a * a, e, e * e, e * f, e * g)]
    var1 = jnp.maximum(saa - sa * sa, 0.0) + eps1
    r = jax.lax.rsqrt(var1)
    m2 = r * (se - sa * sf) + sg
    ms2 = r * (r * (see - sa * (2.0 * sef - sa * sff)) + 2.0 * (seg - sa * sfg)) + sgg
    var2 = jnp.maximum(ms2 - m2 * m2, 0.0) + _EPS
    h3 = ((e - sa * f) * r + (g - m2)) * jax.lax.rsqrt(var2)
    well_conditioned = jnp.logical_and(saa <= _COND * var1, r * r * see + sgg <= _COND * var2)
    redo = jnp.min(jnp.where(well_conditioned, 1, 0)) == 0

    ys = [None] * NT
    gb = [None] * NT

    def tanh_tile(rows, ht):
        if isinstance(rows, int):
            rows = pl.ds(rows * 128, 128)
        v = w1b[rows, :].reshape(16, 8, 128) * ht + b1b[rows, :].reshape(16, 8, 128)
        return jnp.tanh(v * (v * v + k0 / alpha)).reshape(128, 128)

    def reduce_tile(i, t, th):
        part = jnp.dot(ab_v[:, i * 128:(i + 1) * 128].astype(th.dtype), th, preferred_element_type=_F32)
        ys[t] = part if ys[t] is None else part + ys[t]

    def gate_tile(t, r0):
        part = jnp.dot(sc_v[:, r0:r0 + 128].astype(_BF16),
                       wm_v[r0:r0 + 128, 5 * D + t * 128:5 * D + (t + 1) * 128], preferred_element_type=_F32)
        gb[t] = part + gb[t]

    tiles = [(i, t) for i in range(NB) for t in range(NT)]
    n_direct = len(tiles) - _PARK - _LATE
    parked, late = tiles[n_direct:n_direct + _PARK], tiles[n_direct + _PARK:]
    sums = []
    for i, t in tiles[:n_direct]:
        reduce_tile(i, t, tanh_tile(i, h3[:, t * 128:(t + 1) * 128]))
        sums.append(ys[t])
    for k, (i, t) in enumerate(parked):
        ht = jnp.where(sums[n_direct - 2 * _PARK + k] > inf_v[...], 0.0, h3[:, t * 128:(t + 1) * 128])
        th_v[:, k * 128:(k + 1) * 128] = tanh_tile(i, ht)

    gb_cp.wait()
    n = D - _GB_MXU
    for t in range(NT):
        w = wm_v[_GB_MXU:D, 5 * D + t * 128:5 * D + (t + 1) * 128].astype(_F32)
        p3 = (w * scb[...]).reshape(n // 8, 8, 128)
        gb[t] = _allsum8(jnp.sum(p3[:n // 16] + p3[n // 16:], axis=0))

    def unpark(k, i, t):
        reduce_tile(i, t, th_v[:, k * 128:(k + 1) * 128].astype(_BF16))

    pending = [functools.partial(unpark, k, i, t) for k, (i, t) in enumerate(parked)]
    pending += [functools.partial(gate_tile, t, r0) for r0 in range(0, _GB_MXU, 128) for t in range(NT)]
    per = -(-len(pending) // len(late))
    for k, (i, t) in enumerate(late):
        for fn in pending[k * per:(k + 1) * per]:
            fn()
        reduce_tile(i, t, tanh_tile(i, h3[:, t * 128:(t + 1) * 128]))

    def finish(hn, tot):
        lin = lin_v[...]
        outs = []
        for t in range(NT):
            yy = tot[t] + lin
            y = hn[0:1, t * 128:(t + 1) * 128] * (yy[0:1] + yy[1:2]) + (yy[2:3] + yy[3:4])
            outs.append(x1[0:1, t * 128:(t + 1) * 128] + gb[t][0:1] * y)
        o_ref[0] = jnp.concatenate(outs, axis=1).astype(o_ref.dtype)

    finish(h3, ys)

    @pl.when(redo)
    def _():
        hn = _layernorm(_layernorm(x1) * f + g)

        def block(i, tot):
            rows = pl.ds(pl.multiple_of(i * 128, 128), 128)
            return tuple(
                tot[t] + jnp.dot(ab_v[:, rows], tanh_tile(rows, hn[:, t * 128:(t + 1) * 128]),
                                 preferred_element_type=_F32)
                for t in range(NT))

        finish(hn, jax.lax.fori_loop(0, NB, block, (jnp.zeros((8, 128), _F32),) * NT))


@jax.jit
def pallas_adaLN_cond__sliding_block_cached__mixer_token_mlp__decode_kernel(
    A_x: jax.Array,
    A_k_cache: jax.Array,
    A_v_cache: jax.Array,
    A_wq: jax.Array,
    A_wo: jax.Array,
    B_x: jax.Array,
    B_w1: jax.Array,
    B_b1: jax.Array,
    B_w2: jax.Array,
    B_b2: jax.Array,
    c: jax.Array,
    w_mod: jax.Array,
):
    B, Sq, D = A_x.shape
    _, H, Sk, Dh = A_k_cache.shape
    F = B_w1.shape[1]
    assert B == 1 and Sq == 1 and B_w1.shape[0] == 1
    W = min(4096, max(256, Sk // 4))
    HD = H * Dh
    assert A_wq.shape == (D, HD) and W == 4096

    kt = jnp.swapaxes(A_k_cache, 2, 3).reshape(HD, Sk)
    vt = jnp.swapaxes(A_v_cache, 2, 3).reshape(HD, Sk)
    b1 = B_b1.reshape(F // 128, 128)
    w2 = B_w2.reshape(1, F)
    b2 = B_b2.reshape(1, 1)

    NG = H // _GROUP
    scratch = [
        pltpu.VMEM((1, 1, D), _BF16),
        pltpu.VMEM((1, D), _BF16),
        pltpu.VMEM((1, F), _BF16),
        pltpu.VMEM((F // 128, 128), _BF16),
        pltpu.VMEM((1, F), _BF16),
        pltpu.VMEM((1, 1), _BF16),
        pltpu.VMEM((D, 6 * D), _BF16),
        pltpu.VMEM((D, HD), _BF16),
        pltpu.VMEM((HD, D), _BF16),
        pltpu.VMEM((_RING, _CH, W), _BF16),
        pltpu.VMEM((2, _GROUP, _CH), _F32),
        pltpu.VMEM((NG, _GROUP, W), _F32),
        pltpu.VMEM((NG, _GROUP, W), _F32),
        pltpu.VMEM((NG, _GROUP, 128), _F32),
        pltpu.VMEM((_GROUP, D), _F32),
        pltpu.VMEM((8, 5 * D), _F32),
        pltpu.VMEM((8, D), _F32),
        pltpu.VMEM((8, D), _F32),
        pltpu.VMEM((F, 128), _F32),
        pltpu.VMEM((F, 128), _F32),
        pltpu.VMEM((8, F), _F32),
        pltpu.VMEM((8, 128), _F32),
        pltpu.VMEM((D - _GB_MXU, 128), _F32),
        pltpu.VMEM((_NDEF, _CH, 128), _F32),
        pltpu.VMEM((8, D), _F32),
        pltpu.VMEM((128, 128 * _PARK), _F32),
        pltpu.VMEM((8, 128), _F32),
        pltpu.SemaphoreType.DMA((6,)),
        pltpu.SemaphoreType.DMA((_AHEAD,)),
        pltpu.SemaphoreType.DMA((2 * _NU,)),
        pltpu.SemaphoreType.DMA((1,)),
        pltpu.SemaphoreType.DMA((3 * _NDEF,)),
    ]
    return pl.pallas_call(
        functools.partial(_kernel, D=D, H=H, Dh=Dh, Sk=Sk, W=W, F=F),
        out_shape=jax.ShapeDtypeStruct(A_x.shape, A_x.dtype),
        in_specs=[pl.BlockSpec(memory_space=pl.ANY)] * 11,
        out_specs=pl.BlockSpec(memory_space=pltpu.VMEM),
        scratch_shapes=scratch,
        compiler_params=pltpu.CompilerParams(
            vmem_limit_bytes=64 * 1024 * 1024,
            disable_bounds_checks=True,
            disable_semaphore_checks=True),
    )(A_x, kt, vt, A_wq, A_wo, B_w1, b1, w2, b2, c, w_mod)
```
